```python
import jax
import jax.numpy as jnp

def _softmax(x, axis=-1):
    return jax.nn.softmax(x, axis=axis)
def _gelu(x):
    return jax.nn.gelu(x, approximate=True)
def _silu(x):
    return jax.nn.silu(x)
def _sigmoid(x):
    return jax.nn.sigmoid(x)
def _layernorm(x, axis=-1, eps=1e-5):
    m = jnp.mean(x, axis=axis, keepdims=True)
    v = jnp.var(x, axis=axis, keepdims=True)
    return (x - m) / jnp.sqrt(v + eps)
def _scatter_add(tgt, idx, src, axis=0):
    return tgt.at[idx].add(src)
def _segment_sum(src, seg, n):
    return jax.ops.segment_sum(src, seg, n)
class _Rng:
    def __init__(self, key):
        self._k = key
    def _next(self):
        self._k, sub = jax.random.split(self._k)
        return sub
    def normal(self, shape):
        return jax.random.normal(self._next(), shape, dtype=jnp.bfloat16)
    def randint(self, lo, hi, shape):
        return jax.random.randint(self._next(), shape, lo, hi, dtype=jnp.int32)
    def uniform(self, shape, lo=0.0, hi=1.0):
        return jax.random.uniform(self._next(), shape, jnp.bfloat16, lo, hi)
    def permutation(self, n):
        return jax.random.permutation(self._next(), n)


kernel_name = 'gated_mix__compressed_kv_cla__gqa_block_cached__decode'

def setup_inputs():
    _rng = _Rng(jax.random.key(int.from_bytes(__import__("os").urandom(4), "little")))
    _w = (lambda a: (lambda t: t.astype(jnp.bfloat16) if jnp.issubdtype(t.dtype, jnp.floating) else t)(jnp.asarray(a)))
    def _A_setup():
        B, H, Sq, Sk, D, M = 1, 32, 1, 4096, 128, 640
        Dc = 4 * D
        return {
            "x": _w((lambda *s: _rng.normal(s) * 0.05)(B, Sq, M)),
            "c_kv": _w((lambda *s: _rng.normal(s) * 0.05)(B, Sk, Dc)),
            "w_q": _w((lambda *s: _rng.normal(s) * 0.05)(M, H, D) * (M ** -0.5)),
            "w_uk": _w((lambda *s: _rng.normal(s) * 0.05)(Dc, H, D) * (Dc ** -0.5)),
            "w_uv": _w((lambda *s: _rng.normal(s) * 0.05)(Dc, H, D) * (Dc ** -0.5)),
            "w_o": _w((lambda *s: _rng.normal(s) * 0.05)(H, D, M) * ((H * D) ** -0.5)),
        }
    _A_in = _A_setup()

    def _B_setup():
        B, Sq, D = 1, 1, 640
        Hq, Hkv, Sk, Dh = 32, 32, 4096, 128
        assert Hq % Hkv == 0, (Hq, Hkv)
        return {
            "x": _w((lambda *s: _rng.normal(s) * 0.05)(B, Sq, D)),
            "k_cache": _w((lambda *s: _rng.normal(s) * 0.05)(B, Hkv, Sk, Dh)),
            "v_cache": _w((lambda *s: _rng.normal(s) * 0.05)(B, Hkv, Sk, Dh)),
            "wq": _w((lambda *s: _rng.normal(s) * 0.05)(D, Hq * Dh) * (D ** -0.5)),
            "wo": _w((lambda *s: _rng.normal(s) * 0.05)(Hq * Dh, D) * ((Hq * Dh) ** -0.5)),
        }
    _B_in = _B_setup()

    return {
        "A_x": _A_in["x"],
        "A_c_kv": _A_in["c_kv"],
        "A_w_q": _A_in["w_q"],
        "A_w_uk": _A_in["w_uk"],
        "A_w_uv": _A_in["w_uv"],
        "A_w_o": _A_in["w_o"],
        "B_x": _B_in["x"],
        "B_k_cache": _B_in["k_cache"],
        "B_v_cache": _B_in["v_cache"],
        "B_wq": _B_in["wq"],
        "B_wo": _B_in["wo"],
        "gate_w": _w((lambda *s: _rng.normal(s) * 0.05)(640)),
    }

def reference(A_x, A_c_kv, A_w_q, A_w_uk, A_w_uv, A_w_o, B_x, B_k_cache, B_v_cache, B_wq, B_wo, gate_w):
    def _A_ref(x, c_kv, w_q, w_uk, w_uv, w_o):
        B, Sq, M = x.shape[0], x.shape[1], x.shape[2]
        Sk = c_kv.shape[1]
        H, D = w_q.shape[1], w_q.shape[2]
        q = jnp.einsum("bqm,mhd->bhqd", x, w_q)
        k = jnp.einsum("bkc,chd->bhkd", c_kv, w_uk)
        v = jnp.einsum("bkc,chd->bhkd", c_kv, w_uv)
        scores = jnp.einsum("bhqd,bhkd->bhqk", q, k) * (D ** -0.5)
        off = Sk - Sq
        qi = jnp.arange(Sq)[:, None]
        kj = jnp.arange(Sk)[None, :]
        cmask = kj <= (qi + off)
        scores = jnp.where(cmask[None, None], scores, -1e9)
        p = _softmax(scores, axis=-1)
        ctx = jnp.einsum("bhqk,bhkd->bhqd", p, v)
        return jnp.einsum("bhqd,hdm->bqm", ctx, w_o)

    def _B_ref(x, k_cache, v_cache, wq, wo):
        B, Sq, D = x.shape
        Hq, Dh = 32, 128
        Hkv = k_cache.shape[1]
        rep = Hq // Hkv
        q = (lambda x, *d: x.transpose(*d))((x @ wq).reshape(B, Sq, Hq, Dh), 0, 2, 1, 3)
        k = jnp.repeat(k_cache, rep, axis=1)
        v = jnp.repeat(v_cache, rep, axis=1)
        scores = jnp.einsum("bhqd,bhkd->bhqk", q, k) * (Dh ** -0.5)
        p = _softmax(scores, axis=-1)
        o = jnp.einsum("bhqk,bhkd->bhqd", p, v)
        return (lambda x, *d: x.transpose(*d))(o, 0, 2, 1, 3).reshape(B, Sq, Hq * Dh) @ wo

    x = A_x
    g = _sigmoid((x * gate_w).sum(-1, keepdims=True))
    a = _A_ref(x, A_c_kv, A_w_q, A_w_uk, A_w_uv, A_w_o)
    b = _B_ref(x, B_k_cache, B_v_cache, B_wq, B_wo)
    return g * a + (1 - g) * b
```

```python
import functools
import jax
import jax.numpy as jnp
from jax.experimental import pallas as pl
from jax.experimental.pallas import tpu as pltpu

H = 32
D = 128
SK = 4096
M = 640
DC = 512
F32 = jnp.float32
BF16 = jnp.bfloat16
NT = (((1,), (1,)), ((), ()))

KV_CHUNKS = (16, 8, 4, 2, 1, 1)
WO_CHUNKS = (16, 8, 4, 2, 1, 1)


def _starts(chunks):
    out, s = [], 0
    for c in chunks:
        out.append(s)
        s += c
    return out


def _kernel(x_hbm, gate_hbm, ckv_hbm, wqa_hbm, wuk_hbm, wuv_hbm, woa_hbm,
            k_hbm, v_hbm, wqb_hbm, wob_hbm,
            out_ref,
            x_vm, gate_vm, xf_vm, x_smem,
            ckv_vm, wqa_vm, wuk_vm, wuv_vm, woa_vm, k_vm, v_vm, wqb_vm, wob_vm,
            qb_vm, y_vm, s_vm, ctx_vm, sems, *, kv_chunks, wo_chunks):
    nkv = len(kv_chunks)
    nwo = len(wo_chunks)
    kv_s = _starts(kv_chunks)
    wo_s = _starts(wo_chunks)
    scale = D ** -0.5

    cp_x = pltpu.make_async_copy(x_hbm, x_vm, sems.at[0])
    cp_g = pltpu.make_async_copy(gate_hbm, gate_vm, sems.at[1])
    cp_wqb = pltpu.make_async_copy(wqb_hbm, wqb_vm, sems.at[2])
    cp_wqa = pltpu.make_async_copy(wqa_hbm, wqa_vm, sems.at[3])
    cp_wuk = pltpu.make_async_copy(wuk_hbm, wuk_vm, sems.at[4])
    cp_ckv = pltpu.make_async_copy(ckv_hbm, ckv_vm, sems.at[5])
    cp_wuv = pltpu.make_async_copy(wuv_hbm, wuv_vm, sems.at[6])
    cp_woa = pltpu.make_async_copy(woa_hbm, woa_vm, sems.at[7])
    cp_xs = pltpu.make_async_copy(xf_vm, x_smem, sems.at[8])
    base = 9

    def cp_k(i):
        return pltpu.make_async_copy(
            k_hbm.at[pl.ds(kv_s[i], kv_chunks[i])], k_vm.at[pl.ds(kv_s[i], kv_chunks[i])],
            sems.at[base + 2 * i])

    def cp_v(i):
        return pltpu.make_async_copy(
            v_hbm.at[pl.ds(kv_s[i], kv_chunks[i])], v_vm.at[pl.ds(kv_s[i], kv_chunks[i])],
            sems.at[base + 2 * i + 1])

    def cp_wo(i):
        return pltpu.make_async_copy(
            wob_hbm.at[pl.ds(wo_s[i], wo_chunks[i])], wob_vm.at[pl.ds(wo_s[i], wo_chunks[i])],
            sems.at[base + 2 * nkv + i])

    cp_x.start()
    cp_g.start()
    cp_wqb.start()
    cp_wqa.start()
    cp_wuk.start()
    cp_ckv.start()
    cp_wuv.start()
    cp_woa.start()
    for i in range(nkv):
        cp_k(i).start()
        cp_v(i).start()
    for i in range(nwo):
        cp_wo(i).start()

    cp_x.wait()
    cp_g.wait()
    xf = x_vm[...].astype(F32)
    gw = gate_vm[...].astype(F32).reshape(1, M)
    z = jnp.sum(xf * gw, axis=-1, keepdims=True)
    g = 1.0 / (1.0 + jnp.exp(-z))
    xf_vm[...] = xf
    cp_xs.start()

    cp_wqb.wait()
    x8 = jnp.broadcast_to(x_vm[...], (8, M))
    qb = jnp.dot(x8, wqb_vm[...], preferred_element_type=F32) * scale
    for h in range(H):
        qb_vm[h] = qb[:, h * D:(h + 1) * D]

    cp_xs.wait()
    cp_wqa.wait()
    UN = 8

    def qa_body(i, acc):
        for j in range(UN):
            m = i * UN + j
            acc = acc + wqa_vm[m].astype(F32) * x_smem[0, m]
        return acc

    qa = jax.lax.fori_loop(0, M // UN, qa_body, jnp.zeros((H, D), F32))
    qa_b = qa.astype(BF16)

    row = jax.lax.broadcasted_iota(jnp.int32, (H, D), 0)
    lane = jax.lax.broadcasted_iota(jnp.int32, (H, D), 1)
    diag = row == (lane % H)

    cp_wuk.wait()
    sub = jax.lax.broadcasted_iota(jnp.int32, (8, D), 0)

    def ql_body(gi, carry):
        yv = jnp.zeros((8, D), F32)
        for s in range(8):
            t = gi * 8 + s
            wt = jnp.concatenate([wuk_vm[cc * 128 + t] for cc in range(4)], axis=0)
            zt = jax.lax.dot_general(qa_b, wt, NT, preferred_element_type=F32)
            y = jnp.sum(jnp.where(diag, zt, 0.0), axis=0, keepdims=True)
            yv = jnp.where(sub == s, y, yv)
        y_vm[pl.ds(pl.multiple_of(gi * 8, 8), 8), :] = yv
        return carry

    jax.lax.fori_loop(0, 16, ql_body, 0)
    yt = y_vm[...].T
    qlat = jnp.concatenate([yt[cc * H:(cc + 1) * H, :] for cc in range(4)], axis=1)
    qlat_b = (qlat * scale).astype(BF16)

    cp_ckv.wait()
    KB = 512

    def sc_body(i, mx):
        kc = ckv_vm[pl.ds(pl.multiple_of(i * KB, KB), KB), :]
        s = jax.lax.dot_general(qlat_b, kc, NT, preferred_element_type=F32)
        s_vm[i] = s
        return jnp.maximum(mx, s)

    mx = jax.lax.fori_loop(0, SK // KB, sc_body, jnp.full((H, KB), -jnp.inf, F32))
    ma = jnp.max(mx, axis=-1, keepdims=True)

    def cx_body(i, carry):
        acc, lsum = carry
        p = jnp.exp(s_vm[i] - ma)
        kc = ckv_vm[pl.ds(pl.multiple_of(i * KB, KB), KB), :]
        acc = acc + jnp.dot(p.astype(BF16), kc, preferred_element_type=F32)
        return acc, lsum + p

    cl, ls = jax.lax.fori_loop(0, SK // KB, cx_body,
                               (jnp.zeros((H, DC), F32), jnp.zeros((H, KB), F32)))
    la = jnp.sum(ls, axis=-1, keepdims=True)
    cl = cl / la

    cp_wuv.wait()
    u = jnp.concatenate([cl[:, cc * 128:(cc + 1) * 128] for cc in range(4)], axis=0)
    y_vm[...] = u.T

    def cv_body(gi, acc):
        yv = y_vm[pl.ds(pl.multiple_of(gi * 8, 8), 8), :]
        for s in range(8):
            t = gi * 8 + s
            wt = jnp.concatenate([wuv_vm[cc * 128 + t] for cc in range(4)], axis=0)
            lt = jnp.where(diag, jnp.broadcast_to(yv[s:s + 1, :], (H, D)), 0.0).astype(BF16)
            acc = acc + jnp.dot(lt, wt, preferred_element_type=F32)
        return acc

    ctx = jax.lax.fori_loop(0, 16, cv_body, jnp.zeros((H, D), F32))
    for gi in range(4):
        ctx_vm[gi] = ctx[gi * 8:(gi + 1) * 8, :]

    cp_woa.wait()

    def oa_body(h, acc):
        cg = ctx_vm[h // 8]
        lt = jnp.where(sub == h % 8, cg, 0.0).astype(BF16)
        return acc + jnp.dot(lt, woa_vm[h], preferred_element_type=F32)

    a8 = jax.lax.fori_loop(0, H, oa_body, jnp.zeros((8, M), F32))
    a = jnp.sum(a8, axis=0, keepdims=True)

    def head_body(h, carry):
        for i in range(nkv):
            @pl.when(h == kv_s[i])
            def _():
                cp_k(i).wait()
                cp_v(i).wait()
        q = qb_vm[h].astype(BF16)
        s = jax.lax.dot_general(q, k_vm[h], NT, preferred_element_type=F32)
        mh = jnp.max(s, axis=-1, keepdims=True)
        p = jnp.exp(s - mh)
        lh = jnp.sum(p, axis=-1, keepdims=True)
        o = jnp.dot(p.astype(BF16), v_vm[h], preferred_element_type=F32)
        qb_vm[h] = o / lh
        return carry

    jax.lax.fori_loop(0, H, head_body, 0)

    b8 = jnp.zeros((8, M), F32)
    for i in range(nwo):
        cp_wo(i).wait()
        for h in range(wo_s[i], wo_s[i] + wo_chunks[i]):
            b8 = b8 + jnp.dot(qb_vm[h].astype(BF16), wob_vm[h], preferred_element_type=F32)
    out = g * a + (1.0 - g) * b8[0:1, :]
    out_ref[...] = out.astype(out_ref.dtype)


@jax.jit
def pallas_gated_mix__compressed_kv_cla__gqa_block_cached__decode_kernel(
    A_x, A_c_kv, A_w_q, A_w_uk, A_w_uv, A_w_o, B_x, B_k_cache, B_v_cache, B_wq, B_wo, gate_w,
):
    del B_x
    kv_chunks, wo_chunks = KV_CHUNKS, WO_CHUNKS
    nsem = 9 + 2 * len(kv_chunks) + len(wo_chunks)
    hbm = pl.BlockSpec(memory_space=pltpu.HBM)
    out = pl.pallas_call(
        functools.partial(_kernel, kv_chunks=kv_chunks, wo_chunks=wo_chunks),
        out_shape=jax.ShapeDtypeStruct((1, M), BF16),
        in_specs=[hbm] * 11,
        out_specs=pl.BlockSpec(memory_space=pltpu.VMEM),
        scratch_shapes=[
            pltpu.VMEM((1, M), BF16),
            pltpu.VMEM((M,), BF16),
            pltpu.VMEM((1, M), F32),
            pltpu.SMEM((1, M), F32),
            pltpu.VMEM((SK, DC), BF16),
            pltpu.VMEM((M, H, D), BF16),
            pltpu.VMEM((DC, H, D), BF16),
            pltpu.VMEM((DC, H, D), BF16),
            pltpu.VMEM((H, D, M), BF16),
            pltpu.VMEM((H, SK, D), BF16),
            pltpu.VMEM((H, SK, D), BF16),
            pltpu.VMEM((M, H * D), BF16),
            pltpu.VMEM((H, D, M), BF16),
            pltpu.VMEM((H, 8, D), F32),
            pltpu.VMEM((128, 128), F32),
            pltpu.VMEM((SK // 512, H, 512), F32),
            pltpu.VMEM((4, 8, D), F32),
            pltpu.SemaphoreType.DMA((nsem,)),
        ],
        compiler_params=pltpu.CompilerParams(vmem_limit_bytes=112 << 20),
    )(
        A_x.reshape(1, M), gate_w,
        A_c_kv.reshape(SK, DC), A_w_q, A_w_uk, A_w_uv, A_w_o,
        B_k_cache.reshape(H, SK, D), B_v_cache.reshape(H, SK, D),
        B_wq, B_wo.reshape(H, D, M),
    )
    return out.reshape(1, 1, M)
```

```python
import jax
import jax.numpy as jnp
from jax.experimental import pallas as pl
from jax.experimental.pallas import tpu as pltpu

H = 32
D = 128
SK = 4096
M = 640
DC = 512
KB = 512
F32 = jnp.float32
BF16 = jnp.bfloat16
NT = (((1,), (1,)), ((), ()))

V_CHUNKS = (24, 8)
WO_MXU_CHUNKS = (16, 12, 2)
WO_VPU_CHUNKS = (128, 96, 32)


def _starts(chunks, first=0):
    out = []
    for c in chunks:
        out.append(first)
        first += c
    return out


def _kernel(x_hbm, gate_hbm, ckv_hbm, wqa_hbm, wuk_hbm, wuv_hbm, woa_hbm,
            k_hbm, v_hbm, wqb_hbm, wob_hbm,
            out_ref,
            x_vm, gate_vm, xf_vm, x_smem,
            ckv_vm, wqa_vm, wuk_vm, wuv_vm, woa_vm, k_vm, v_vm, wqb_vm, wob_vm,
            qb_vm, p_vm, l_vm, o_vm, ot_vm, y_vm, s_vm, ctx_vm, sems):
    scale = D ** -0.5

    copies = {}

    def add(name, src, dst):
        copies[name] = pltpu.make_async_copy(src, dst, sems.at[len(copies)])

    add("wqb", wqb_hbm, wqb_vm)
    add("x", x_hbm, x_vm)
    add("gate", gate_hbm, gate_vm)
    add("wqa", wqa_hbm, wqa_vm)
    add("wuk", wuk_hbm, wuk_vm)
    add("ckv", ckv_hbm, ckv_vm)
    add("wuv", wuv_hbm, wuv_vm)
    add("woa", woa_hbm, woa_vm)
    add("k", k_hbm, k_vm)
    v_start = _starts(V_CHUNKS)
    for i, (s, n) in enumerate(zip(v_start, V_CHUNKS)):
        add(("v", i), v_hbm.at[pl.ds(s, n)], v_vm.at[pl.ds(s, n)])
    wo_start = _starts(WO_MXU_CHUNKS)
    for i, (s, n) in enumerate(zip(wo_start, WO_MXU_CHUNKS)):
        rows = pl.ds(s * D, n * D)
        add(("wo", i), wob_hbm.at[rows], wob_vm.at[rows])
    vpu_head0 = sum(WO_MXU_CHUNKS)
    vpu_row0 = vpu_head0 * D
    vpu_start = _starts(WO_VPU_CHUNKS, vpu_row0)
    for i, (s, n) in enumerate(zip(vpu_start, WO_VPU_CHUNKS)):
        add(("wo_vpu", i), wob_hbm.at[pl.ds(s, n)], wob_vm.at[pl.ds(s, n)])
    for c in copies.values():
        c.start()
    x_to_smem = pltpu.make_async_copy(xf_vm, x_smem, sems.at[len(copies)])

    sub = jax.lax.broadcasted_iota(jnp.int32, (8, D), 0)
    row = jax.lax.broadcasted_iota(jnp.int32, (H, D), 0)
    lane = jax.lax.broadcasted_iota(jnp.int32, (H, D), 1)
    diag = row == lane % H

    copies["x"].wait()
    copies["gate"].wait()
    xf = x_vm[...].astype(F32)
    xf_vm[...] = xf
    x_to_smem.start()
    gw = gate_vm[...].astype(F32).reshape(1, M)
    z = jnp.sum(xf * gw, axis=-1, keepdims=True)
    g = 1.0 / (1.0 + jnp.exp(-z))

    copies["wqb"].wait()
    x8 = jnp.broadcast_to(x_vm[...], (8, M))
    qb = jnp.dot(x8, wqb_vm[...], preferred_element_type=F32) * scale
    for h in range(H):
        qb_vm[h] = jnp.where(sub == h % 8, qb[:, h * D:(h + 1) * D], 0.0)

    x_to_smem.wait()
    copies["wqa"].wait()

    def qa_body(i, acc):
        for j in range(8):
            m = i * 8 + j
            acc = acc + wqa_vm[m].astype(F32) * x_smem[0, m]
        return acc

    qa = jax.lax.fori_loop(0, M // 8, qa_body, jnp.zeros((H, D), F32)).astype(BF16)

    copies["wuk"].wait()

    def qlat_body(i, carry):
        rows8 = jnp.zeros((8, D), F32)
        for j in range(8):
            t = i * 8 + j
            w = jnp.concatenate([wuk_vm[cc * D + t] for cc in range(DC // D)], axis=0)
            prod = jax.lax.dot_general(qa, w, NT, preferred_element_type=F32)
            picked = jnp.sum(jnp.where(diag, prod, 0.0), axis=0, keepdims=True)
            rows8 = jnp.where(sub == j, picked, rows8)
        y_vm[pl.ds(pl.multiple_of(i * 8, 8), 8), :] = rows8
        return carry

    jax.lax.fori_loop(0, D // 8, qlat_body, 0)
    yt = y_vm[...].T
    qlat = jnp.concatenate([yt[cc * H:(cc + 1) * H, :] for cc in range(DC // D)], axis=1)
    qlat = (qlat * scale).astype(BF16)

    copies["ckv"].wait()

    def score_body(i, mx):
        c = ckv_vm[pl.ds(pl.multiple_of(i * KB, KB), KB), :]
        s = jax.lax.dot_general(qlat, c, NT, preferred_element_type=F32)
        s_vm[i] = s
        return jnp.maximum(mx, s)

    mx = jax.lax.fori_loop(0, SK // KB, score_body, jnp.full((H, KB), -jnp.inf, F32))
    ma = jnp.max(mx, axis=-1, keepdims=True)

    def ctx_lat_body(i, carry):
        acc, lsum = carry
        p = jnp.exp(s_vm[i] - ma)
        c = ckv_vm[pl.ds(pl.multiple_of(i * KB, KB), KB), :]
        return acc + jnp.dot(p.astype(BF16), c, preferred_element_type=F32), lsum + p

    clat, lsum = jax.lax.fori_loop(
        0, SK // KB, ctx_lat_body, (jnp.zeros((H, DC), F32), jnp.zeros((H, KB), F32)))
    clat = clat / jnp.sum(lsum, axis=-1, keepdims=True)

    copies["wuv"].wait()
    u = jnp.concatenate([clat[:, cc * D:(cc + 1) * D] for cc in range(DC // D)], axis=0)
    y_vm[...] = u.T

    def ctx_body(i, acc):
        rows8 = y_vm[pl.ds(pl.multiple_of(i * 8, 8), 8), :]
        for j in range(8):
            t = i * 8 + j
            w = jnp.concatenate([wuv_vm[cc * D + t] for cc in range(DC // D)], axis=0)
            lhs = jnp.where(diag, jnp.broadcast_to(rows8[j:j + 1, :], (H, D)), 0.0)
            acc = acc + jnp.dot(lhs.astype(BF16), w, preferred_element_type=F32)
        return acc

    ctx = jax.lax.fori_loop(0, D // 8, ctx_body, jnp.zeros((H, D), F32))
    for i in range(H // 8):
        ctx_vm[i] = ctx[i * 8:(i + 1) * 8, :]

    copies["woa"].wait()

    def proj_a_body(h, acc):
        lhs = jnp.where(sub == h % 8, ctx_vm[h // 8], 0.0)
        return acc + jnp.dot(lhs.astype(BF16), woa_vm[h], preferred_element_type=F32)

    a8 = jax.lax.fori_loop(0, H, proj_a_body, jnp.zeros((8, M), F32))
    ga = g * jnp.sum(a8, axis=0, keepdims=True)

    copies["k"].wait()

    def softmax_b_body(i, carry):
        s = jnp.zeros((8, SK), F32)
        for j in range(8):
            h = i * 8 + j
            s = s + jax.lax.dot_general(qb_vm[h].astype(BF16), k_vm[h], NT,
                                        preferred_element_type=F32)
        p = jnp.exp(s - jnp.max(s, axis=-1, keepdims=True))
        l_vm[i] = jnp.broadcast_to(jnp.sum(p, axis=-1, keepdims=True), (8, D))
        p_vm[i] = p.astype(BF16)
        return carry

    jax.lax.fori_loop(0, H // 8, softmax_b_body, 0)

    omg = 1.0 - g

    def pv_body(h, carry):
        o = jnp.dot(p_vm[h // 8], v_vm[h], preferred_element_type=F32)
        o = o * (omg / l_vm[h // 8])
        o = jnp.sum(jnp.where(sub == h % 8, o, 0.0), axis=0, keepdims=True)
        o_vm[h] = jnp.broadcast_to(o, (8, D))
        return carry

    for i, (s, n) in enumerate(zip(v_start, V_CHUNKS)):
        copies[("v", i)].wait()
        jax.lax.fori_loop(s, s + n, pv_body, 0)

    for j in range(H - vpu_head0):
        ot_vm[pl.ds(j * D, D), :] = jnp.broadcast_to(o_vm[vpu_head0 + j][0:1, :], (D, D)).T
    b8 = jnp.zeros((8, M), F32)
    for i, (s, n) in enumerate(zip(wo_start, WO_MXU_CHUNKS)):
        copies[("wo", i)].wait()
        for h in range(s, s + n):
            b8 = b8 + jnp.dot(o_vm[h].astype(BF16), wob_vm[pl.ds(h * D, D), :],
                              preferred_element_type=F32)
    out = ga + b8[0:1, :]
    for i, (s, n) in enumerate(zip(vpu_start, WO_VPU_CHUNKS)):
        copies[("wo_vpu", i)].wait()
        w = wob_vm[pl.ds(s, n), :].astype(F32)
        o_col = ot_vm[pl.ds(s - vpu_row0, n), :]
        o_col = jnp.concatenate([o_col] * (M // D), axis=1)
        out = out + jnp.sum(w * o_col, axis=0, keepdims=True)
    out_ref[...] = out.astype(out_ref.dtype)


def _forward(A_x, A_c_kv, A_w_q, A_w_uk, A_w_uv, A_w_o, B_k_cache, B_v_cache, B_wq, B_wo,
             gate_w, interpret=False):
    n_copies = 9 + len(V_CHUNKS) + len(WO_MXU_CHUNKS) + len(WO_VPU_CHUNKS)
    vpu_rows = sum(WO_VPU_CHUNKS)
    hbm = pl.BlockSpec(memory_space=pltpu.HBM)
    out = pl.pallas_call(
        _kernel,
        out_shape=jax.ShapeDtypeStruct((1, M), A_x.dtype),
        in_specs=[hbm] * 11,
        out_specs=pl.BlockSpec(memory_space=pltpu.VMEM),
        scratch_shapes=[
            pltpu.VMEM((1, M), BF16),
            pltpu.VMEM((M,), BF16),
            pltpu.VMEM((1, M), F32),
            pltpu.SMEM((1, M), F32),
            pltpu.VMEM((SK, DC), BF16),
            pltpu.VMEM((M, H, D), BF16),
            pltpu.VMEM((DC, H, D), BF16),
            pltpu.VMEM((DC, H, D), BF16),
            pltpu.VMEM((H, D, M), BF16),
            pltpu.VMEM((H, SK, D), BF16),
            pltpu.VMEM((H, SK, D), BF16),
            pltpu.VMEM((M, H * D), BF16),
            pltpu.VMEM((H * D, M), BF16),
            pltpu.VMEM((H, 8, D), F32),
            pltpu.VMEM((H // 8, 8, SK), BF16),
            pltpu.VMEM((H // 8, 8, D), F32),
            pltpu.VMEM((H, 8, D), F32),
            pltpu.VMEM((vpu_rows, D), F32),
            pltpu.VMEM((D, D), F32),
            pltpu.VMEM((SK // KB, H, KB), F32),
            pltpu.VMEM((H // 8, 8, D), F32),
            pltpu.SemaphoreType.DMA((n_copies + 1,)),
        ],
        compiler_params=pltpu.CompilerParams(
            vmem_limit_bytes=112 << 20,
            disable_semaphore_checks=True,
        ),
        interpret=interpret,
    )(
        A_x.reshape(1, M), gate_w,
        A_c_kv.reshape(SK, DC), A_w_q, A_w_uk, A_w_uv, A_w_o,
        B_k_cache.reshape(H, SK, D), B_v_cache.reshape(H, SK, D),
        B_wq, B_wo,
    )
    return out.reshape(1, 1, M)


@jax.jit
def pallas_gated_mix__compressed_kv_cla__gqa_block_cached__decode_kernel(
    A_x: jax.Array,
    A_c_kv: jax.Array,
    A_w_q: jax.Array,
    A_w_uk: jax.Array,
    A_w_uv: jax.Array,
    A_w_o: jax.Array,
    B_x: jax.Array,
    B_k_cache: jax.Array,
    B_v_cache: jax.Array,
    B_wq: jax.Array,
    B_wo: jax.Array,
    gate_w: jax.Array,
):
    del B_x
    return _forward(A_x, A_c_kv, A_w_q, A_w_uk, A_w_uv, A_w_o,
                    B_k_cache, B_v_cache, B_wq, B_wo, gate_w)
```

```python
import functools

import jax
import jax.numpy as jnp
from jax.experimental import pallas as pl
from jax.experimental.pallas import tpu as pltpu

H = 32
D = 128
SK = 4096
M = 640
DC = 512
KB = 512
F32 = jnp.float32
BF16 = jnp.bfloat16
NT = (((1,), (1,)), ((), ()))

KV_ROWS = 128
WO_ROWS = 32

S_X, S_GATE, S_XS, S_WQB, S_WQA, S_WUK, S_CKV, S_WUV, S_WOA = range(9)
S_K = 9
S_V = S_K + 4
S_WOB = S_V + H


def _kernel(*refs, cfg):
    n_sems = S_WOB + 1 + len(cfg['wob_b_units'])
    pl.run_scoped(functools.partial(_body, *refs, cfg=cfg), pltpu.SemaphoreType.DMA((n_sems,)))


def _body(x_hbm, gate_hbm, ckv_hbm, wqa_hbm, wuk_hbm, wuv_hbm, woa_hbm,
          k_hbm, v_hbm, wqb_hbm, wob_hbm,
          out_ref,
          x_vm, gate_vm, xf_vm, x_smem,
          ckv_vm, wqa_vm, wuk_vm, wuv_vm, woa_vm, k_vm, v_vm, wqb_vm, wob_vm,
          qb_vm, sb_vm, p_vm, l_vm, o_vm, ot_vm, y_vm, s_vm, ctx_vm, sems, *, cfg):
    scale = D ** -0.5

    def start(src, dst, sem, thread):
        pltpu.make_async_copy(src, dst, sems.at[sem]).start(thread)

    def wait_all(buf, sem):
        pltpu.make_async_copy(buf, buf, sems.at[sem]).wait()

    def pair_lead(hbm, vm, half, n, j, sem):
        for t in range(2):
            sl = pl.ds(t * half + j * n, n)
            start(hbm.at[sl], vm.at[sl], sem, t)

    def pair_wqb(j):
        r, c = (j // 2) * 8, (j % 2) * 2048
        for t in range(2):
            idx = (pl.ds(t * (M // 2) + r, 8), pl.ds(c, 2048))
            start(wqb_hbm.at[idx], wqb_vm.at[idx], S_WQB, t)

    weight_pairs = (
        [functools.partial(pair_wqb, j) for j in range(80)]
        + [functools.partial(pair_lead, wqa_hbm, wqa_vm, M // 2, 4, j, S_WQA) for j in range(80)]
        + [functools.partial(pair_lead, wuk_hbm, wuk_vm, DC // 2, 4, j, S_WUK) for j in range(64)]
        + [functools.partial(pair_lead, ckv_hbm, ckv_vm, SK // 2, 32, j, S_CKV) for j in range(64)]
        + [functools.partial(pair_lead, wuv_hbm, wuv_vm, DC // 2, 4, j, S_WUV) for j in range(64)]
        + [functools.partial(pair_lead, woa_hbm, woa_vm, H * D // 2, WO_ROWS, j, S_WOA) for j in range(64)]
    )
    issued = [0]

    def pump_weights(n):
        for f in weight_pairs[issued[0]:issued[0] + n]:
            f()
        issued[0] += n

    HALF = H * SK // 2
    PPH = SK // KV_ROWS

    def pair_k(j):
        g = j // (8 * PPH)
        for t in range(2):
            sl = pl.ds(pl.multiple_of(t * HALF + j * KV_ROWS, KV_ROWS), KV_ROWS)
            start(k_hbm.at[sl], k_vm.at[sl], S_K + 2 * t + g, t)

    def pair_v(j):
        h = j // PPH
        for t in range(2):
            sl = pl.ds(pl.multiple_of(t * HALF + j * KV_ROWS, KV_ROWS), KV_ROWS)
            start(v_hbm.at[sl], v_vm.at[sl], S_V + 16 * t + h, t)

    b_units = cfg['wob_b_units']
    b_unit_of_chunk = []
    for u, rows in enumerate(b_units):
        b_unit_of_chunk += [u] * (rows // WO_ROWS)
    assert len(b_unit_of_chunk) == 64

    def pair_wob(j):
        sl = pl.ds(j * WO_ROWS, WO_ROWS)
        start(wob_hbm.at[sl], wob_vm.at[sl], S_WOB, 0)
        sl = pl.ds(H * D // 2 + j * WO_ROWS, WO_ROWS)
        start(wob_hbm.at[sl], wob_vm.at[sl], S_WOB + 1 + b_unit_of_chunk[j], 1)

    def pump_loop(pair_fn, j0, n):
        step = 8 if n % 8 == 0 else (4 if n % 4 == 0 else 1)

        def body(i, c):
            for jj in range(step):
                pair_fn(j0 + i * step + jj)
            return c
        jax.lax.fori_loop(0, n // step, body, 0)

    start(x_hbm, x_vm, S_X, 0)
    start(gate_hbm, gate_vm, S_GATE, 0)
    pump_weights(160)

    sub = jax.lax.broadcasted_iota(jnp.int32, (8, D), 0)
    row = jax.lax.broadcasted_iota(jnp.int32, (H, D), 0)
    lane = jax.lax.broadcasted_iota(jnp.int32, (H, D), 1)
    diag = row == lane % H

    pltpu.make_async_copy(x_hbm, x_vm, sems.at[S_X]).wait()
    pltpu.make_async_copy(gate_hbm, gate_vm, sems.at[S_GATE]).wait()
    xf = x_vm[...].astype(F32)
    xf_vm[...] = xf
    start(xf_vm, x_smem, S_XS, 0)
    gw = gate_vm[...].astype(F32).reshape(1, M)
    z = jnp.sum(xf * gw, axis=-1, keepdims=True)
    g = 1.0 / (1.0 + jnp.exp(-z))

    wait_all(wqb_vm, S_WQB)
    x8 = jnp.broadcast_to(x_vm[...], (8, M))
    qb = jnp.dot(x8, wqb_vm[...], preferred_element_type=F32) * scale
    for h in range(H):
        qb_vm[h] = jnp.where(sub == h % 8, qb[:, h * D:(h + 1) * D], 0.0)
    pump_weights(80)

    pltpu.make_async_copy(xf_vm, x_smem, sems.at[S_XS]).wait()
    wait_all(wqa_vm, S_WQA)

    def qa_body(i, acc):
        for j in range(8):
            m = i * 8 + j
            acc = acc + wqa_vm[m].astype(F32) * x_smem[0, m]
        return acc

    qa = jax.lax.fori_loop(0, M // 8, qa_body, jnp.zeros((H, D), F32)).astype(BF16)
    pump_weights(64)

    wait_all(wuk_vm, S_WUK)

    def qlat_body(i, carry):
        rows8 = jnp.zeros((8, D), F32)
        for j in range(8):
            t = i * 8 + j
            w = jnp.concatenate([wuk_vm[cc * D + t] for cc in range(DC // D)], axis=0)
            prod = jax.lax.dot_general(qa, w, NT, preferred_element_type=F32)
            picked = jnp.sum(jnp.where(diag, prod, 0.0), axis=0, keepdims=True)
            rows8 = jnp.where(sub == j, picked, rows8)
        y_vm[pl.ds(pl.multiple_of(i * 8, 8), 8), :] = rows8
        return carry

    jax.lax.fori_loop(0, D // 8, qlat_body, 0)
    yt = y_vm[...].T
    qlat = jnp.concatenate([yt[cc * H:(cc + 1) * H, :] for cc in range(DC // D)], axis=1)
    qlat = (qlat * scale).astype(BF16)
    pump_weights(64)

    wait_all(ckv_vm, S_CKV)

    def score_body(i, mx):
        c = ckv_vm[pl.ds(pl.multiple_of(i * KB, KB), KB), :]
        s = jax.lax.dot_general(qlat, c, NT, preferred_element_type=F32)
        s_vm[i] = s
        return jnp.maximum(mx, s)

    mx = jax.lax.fori_loop(0, SK // KB, score_body, jnp.full((H, KB), -jnp.inf, F32))
    ma = jnp.max(mx, axis=-1, keepdims=True)
    pump_weights(24)

    def ctx_lat_body(i, carry):
        acc, lsum = carry
        p = jnp.exp(s_vm[i] - ma)
        c = ckv_vm[pl.ds(pl.multiple_of(i * KB, KB), KB), :]
        return acc + jnp.dot(p.astype(BF16), c, preferred_element_type=F32), lsum + p

    clat, lsum = jax.lax.fori_loop(
        0, SK // KB, ctx_lat_body, (jnp.zeros((H, DC), F32), jnp.zeros((H, KB), F32)))
    clat = clat / jnp.sum(lsum, axis=-1, keepdims=True)
    pump_weights(24)
    assert issued[0] == len(weight_pairs)
    pump_loop(pair_k, 0, 16)

    wait_all(wuv_vm, S_WUV)
    u = jnp.concatenate([clat[:, cc * D:(cc + 1) * D] for cc in range(DC // D)], axis=0)
    y_vm[...] = u.T

    def ctx_body(i, acc):
        rows8 = y_vm[pl.ds(pl.multiple_of(i * 8, 8), 8), :]
        for j in range(8):
            t = i * 8 + j
            w = jnp.concatenate([wuv_vm[cc * D + t] for cc in range(DC // D)], axis=0)
            lhs = jnp.where(diag, jnp.broadcast_to(rows8[j:j + 1, :], (H, D)), 0.0)
            acc = acc + jnp.dot(lhs.astype(BF16), w, preferred_element_type=F32)
        return acc

    ctx = jax.lax.fori_loop(0, D // 8, ctx_body, jnp.zeros((H, D), F32))
    for i in range(H // 8):
        ctx_vm[i] = ctx[i * 8:(i + 1) * 8, :]
    pump_loop(pair_k, 16, 64)

    wait_all(woa_vm, S_WOA)

    def proj_a_body(h, acc):
        lhs = jnp.where(sub == h % 8, ctx_vm[h // 8], 0.0)
        w = woa_vm[pl.ds(pl.multiple_of(h * D, D), D), :]
        return acc + jnp.dot(lhs.astype(BF16), w, preferred_element_type=F32)

    a8 = jax.lax.fori_loop(0, H, proj_a_body, jnp.zeros((8, M), F32))
    ga = g * jnp.sum(a8, axis=0, keepdims=True)
    pump_loop(pair_k, 80, 256)

    def qk_group(g_idx, pair_fn, j0, n):
        wait_all(k_vm.at[pl.ds(g_idx * 8 * SK, 8 * SK)], K_SEM_OF_GROUP[g_idx])
        sb_vm[...] = jnp.zeros((8, SK), F32)

        def body(j, c):
            for jj in range(n):
                pair_fn(j0 + j * n + jj)
            h = g_idx * 8 + j
            kh = k_vm[pl.ds(pl.multiple_of(h * SK, SK), SK), :]
            sb_vm[...] += jax.lax.dot_general(qb_vm[h].astype(BF16), kh, NT,
                                              preferred_element_type=F32)
            return c
        jax.lax.fori_loop(0, 8, body, 0)
        s = sb_vm[...]
        p = jnp.exp(s - jnp.max(s, axis=-1, keepdims=True))
        l_vm[g_idx] = jnp.broadcast_to(jnp.sum(p, axis=-1, keepdims=True), (8, D))
        p_vm[g_idx] = p.astype(BF16)

    K_SEM_OF_GROUP = [S_K + 0, S_K + 1, S_K + 2, S_K + 3]
    qk_group(0, pair_k, 336, 11)
    qk_group(2, pair_k, 424, 11)
    pump_loop(pair_v, 0, 80)
    qk_group(1, pair_v, 80, 11)
    qk_group(3, pair_v, 168, 11)

    omg = 1.0 - g

    def pv_head(h):
        wait_all(v_vm.at[pl.ds(pl.multiple_of(h * SK, SK), SK)], S_V + h)
        vh = v_vm[pl.ds(pl.multiple_of(h * SK, SK), SK), :]
        o = jnp.dot(p_vm[h // 8], vh, preferred_element_type=F32)
        o = o * (omg / l_vm[h // 8])
        o = jnp.sum(jnp.where(sub == h % 8, o, 0.0), axis=0, keepdims=True)
        o_vm[h] = jnp.broadcast_to(o, (8, D))

    def pv_loop1(i, c):
        for jj in range(32):
            pair_v(256 + i * 32 + jj)
        pv_head(i)
        pv_head(16 + i)
        return c
    jax.lax.fori_loop(0, 8, pv_loop1, 0)
    for i in range(8, 16):
        for jj in range(8):
            pair_wob((i - 8) * 8 + jj)
        pv_head(i)
        pv_head(16 + i)

    vpu_units = cfg['vpu_units']
    n_mxu_units = len(b_units) - vpu_units
    b_starts = [H * D // 2]
    for rows in b_units:
        b_starts.append(b_starts[-1] + rows)
    vpu_row0 = b_starts[n_mxu_units]
    assert vpu_row0 % D == 0
    vpu_head0 = vpu_row0 // D
    for j in range(H - vpu_head0):
        ot_vm[pl.ds(j * D, D), :] = jnp.broadcast_to(o_vm[vpu_head0 + j][0:1, :], (D, D)).T
    b8 = jnp.zeros((8, M), F32)

    def proj_heads(b8, h0, h1):
        for h in range(h0, h1):
            b8 = b8 + jnp.dot(o_vm[h].astype(BF16), wob_vm[pl.ds(h * D, D), :],
                              preferred_element_type=F32)
        return b8

    wait_all(wob_vm.at[pl.ds(0, H * D // 2)], S_WOB)
    b8 = proj_heads(b8, 0, H // 2)
    for u in range(n_mxu_units):
        r0, n = b_starts[u], b_units[u]
        wait_all(wob_vm.at[pl.ds(r0, n)], S_WOB + 1 + u)
        assert r0 % D == 0 and n % D == 0
        b8 = proj_heads(b8, r0 // D, (r0 + n) // D)
    out = ga + b8[0:1, :]
    for u in range(n_mxu_units, len(b_units)):
        s, n = b_starts[u], b_units[u]
        wait_all(wob_vm.at[pl.ds(s, n)], S_WOB + 1 + u)
        w = wob_vm[pl.ds(s, n), :].astype(F32)
        o_col = ot_vm[pl.ds(s - vpu_row0, n), :]
        o_col = jnp.concatenate([o_col] * (M // D), axis=1)
        out = out + jnp.sum(w * o_col, axis=0, keepdims=True)
    out_ref[...] = out.astype(out_ref.dtype)


CFG = dict(wob_b_units=(12 * 128, 2 * 128, 128, 96, 32), vpu_units=3)


def _forward(A_x, A_c_kv, A_w_q, A_w_uk, A_w_uv, A_w_o, B_k_cache, B_v_cache, B_wq, B_wo,
             gate_w, interpret=False):
    cfg = CFG
    vpu_rows = sum(cfg['wob_b_units'][len(cfg['wob_b_units']) - cfg['vpu_units']:])
    hbm = pl.BlockSpec(memory_space=pltpu.HBM)
    out = pl.pallas_call(
        functools.partial(_kernel, cfg=cfg),
        out_shape=jax.ShapeDtypeStruct((1, M), A_x.dtype),
        in_specs=[hbm] * 11,
        out_specs=pl.BlockSpec(memory_space=pltpu.VMEM),
        scratch_shapes=[
            pltpu.VMEM((1, M), BF16),
            pltpu.VMEM((M,), BF16),
            pltpu.VMEM((1, M), F32),
            pltpu.SMEM((1, M), F32),
            pltpu.VMEM((SK, DC), BF16),
            pltpu.VMEM((M, H, D), BF16),
            pltpu.VMEM((DC, H, D), BF16),
            pltpu.VMEM((DC, H, D), BF16),
            pltpu.VMEM((H * D, M), BF16),
            pltpu.VMEM((H * SK, D), BF16),
            pltpu.VMEM((H * SK, D), BF16),
            pltpu.VMEM((M, H * D), BF16),
            pltpu.VMEM((H * D, M), BF16),
            pltpu.VMEM((H, 8, D), F32),
            pltpu.VMEM((8, SK), F32),
            pltpu.VMEM((H // 8, 8, SK), BF16),
            pltpu.VMEM((H // 8, 8, D), F32),
            pltpu.VMEM((H, 8, D), F32),
            pltpu.VMEM((vpu_rows, D), F32),
            pltpu.VMEM((D, D), F32),
            pltpu.VMEM((SK // KB, H, KB), F32),
            pltpu.VMEM((H // 8, 8, D), F32),
        ],
        compiler_params=pltpu.CompilerParams(vmem_limit_bytes=112 << 20),
        interpret=interpret,
    )(
        A_x.reshape(1, M), gate_w,
        A_c_kv.reshape(SK, DC), A_w_q, A_w_uk, A_w_uv, A_w_o.reshape(H * D, M),
        B_k_cache.reshape(H * SK, D), B_v_cache.reshape(H * SK, D),
        B_wq, B_wo,
    )
    return out.reshape(1, 1, M)


@jax.jit
def pallas_gated_mix__compressed_kv_cla__gqa_block_cached__decode_kernel(
    A_x: jax.Array,
    A_c_kv: jax.Array,
    A_w_q: jax.Array,
    A_w_uk: jax.Array,
    A_w_uv: jax.Array,
    A_w_o: jax.Array,
    B_x: jax.Array,
    B_k_cache: jax.Array,
    B_v_cache: jax.Array,
    B_wq: jax.Array,
    B_wo: jax.Array,
    gate_w: jax.Array,
):
    del B_x
    return _forward(A_x, A_c_kv, A_w_q, A_w_uk, A_w_uv, A_w_o,
                    B_k_cache, B_v_cache, B_wq, B_wo, gate_w)
```

```python
import functools

import jax
import jax.numpy as jnp
from jax.experimental import pallas as pl
from jax.experimental.pallas import tpu as pltpu

H = 32
D = 128
SK = 4096
M = 640
DC = 512
KB = 512
F32 = jnp.float32
BF16 = jnp.bfloat16
NT = (((1,), (1,)), ((), ()))

KV_ROWS = 128
WO_ROWS = 32

S_X, S_GATE, S_XS, S_WQB, S_WQA, S_WUK, S_CKV, S_WUV, S_WOA = range(9)
S_K = 9
S_V = S_K + 4
S_WOB = S_V + H


def _kernel(*refs, cfg):
    n_sems = S_WOB + 1 + len(cfg['wob_b_units'])
    pl.run_scoped(functools.partial(_body, *refs, cfg=cfg), pltpu.SemaphoreType.DMA((n_sems,)))


def _body(x_hbm, gate_hbm, ckv_hbm, wqa_hbm, wuk_hbm, wuv_hbm, woa_hbm,
          k_hbm, v_hbm, wqb_hbm, wob_hbm,
          out_ref,
          x_vm, gate_vm, xf_vm, x_smem,
          ckv_vm, wqa_vm, wuk_vm, wuv_vm, woa_vm, k_vm, v_vm, wqb_vm, wob_vm,
          qb_vm, sb_vm, p_vm, l_vm, o_vm, ot_vm, y_vm, s_vm, ctx_vm, sems, *, cfg):
    scale = D ** -0.5
    compute = cfg['compute']
    import contextlib
    def scope(name):
        return jax.named_scope(name) if cfg.get('scopes') else contextlib.nullcontext()

    def start(src, dst, sem, thread):
        pltpu.make_async_copy(src, dst, sems.at[sem]).start(thread)

    def wait_all(buf, sem, name=None):
        if name is None:
            pltpu.make_async_copy(buf, buf, sems.at[sem]).wait()
        else:
            with scope('wait_' + name):
                pltpu.make_async_copy(buf, buf, sems.at[sem]).wait()

    def pair_lead(hbm, vm, half, n, j, sem):
        for t in range(2):
            off = t * half + j * n
            sl = pl.ds(off if isinstance(off, int) else pl.multiple_of(off, n), n)
            start(hbm.at[sl], vm.at[sl], sem, t)

    def pair_wqb(j):
        r, c = (j // 2) * 8, (j % 2) * 2048
        for t in range(2):
            idx = (pl.ds(t * (M // 2) + r, 8), pl.ds(c, 2048))
            start(wqb_hbm.at[idx], wqb_vm.at[idx], S_WQB, t)

    weight_pairs = (
        [functools.partial(pair_wqb, j) for j in range(80)]
        + [functools.partial(pair_lead, wqa_hbm, wqa_vm, M // 2, 4, j, S_WQA) for j in range(80)]
        + [functools.partial(pair_lead, wuk_hbm, wuk_vm, DC // 2, 4, j, S_WUK) for j in range(64)]
        + [functools.partial(pair_lead, ckv_hbm, ckv_vm, SK // 2, 32, j, S_CKV) for j in range(64)]
        + [functools.partial(pair_lead, wuv_hbm, wuv_vm, DC // 2, 4, j, S_WUV) for j in range(64)]
        + [functools.partial(pair_lead, woa_hbm, woa_vm, H * D // 2, WO_ROWS, j, S_WOA) for j in range(64)]
    )
    issued = [0]

    def pump_weights(n):
        with scope(f'pumpW_{issued[0]}'):
            for f in weight_pairs[issued[0]:issued[0] + n]:
                f()
        issued[0] += n

    HALF = H * SK // 2
    PPH = SK // KV_ROWS

    def pair_k(j):
        g = j // (8 * PPH)
        for t in range(2):
            sl = pl.ds(pl.multiple_of(t * HALF + j * KV_ROWS, KV_ROWS), KV_ROWS)
            start(k_hbm.at[sl], k_vm.at[sl], S_K + 2 * t + g, t)

    def pair_v(j):
        h = j // PPH
        for t in range(2):
            sl = pl.ds(pl.multiple_of(t * HALF + j * KV_ROWS, KV_ROWS), KV_ROWS)
            start(v_hbm.at[sl], v_vm.at[sl], S_V + 16 * t + h, t)

    b_units = cfg['wob_b_units']
    b_unit_of_chunk = []
    for u, rows in enumerate(b_units):
        b_unit_of_chunk += [u] * (rows // WO_ROWS)
    assert len(b_unit_of_chunk) == 64

    def pair_wob(j):
        sl = pl.ds(j * WO_ROWS, WO_ROWS)
        start(wob_hbm.at[sl], wob_vm.at[sl], S_WOB, 0)
        sl = pl.ds(H * D // 2 + j * WO_ROWS, WO_ROWS)
        start(wob_hbm.at[sl], wob_vm.at[sl], S_WOB + 1 + b_unit_of_chunk[j], 1)

    def pump_loop(pair_fn, j0, n):
        step = 8 if n % 8 == 0 else (4 if n % 4 == 0 else 1)

        def body(i, c):
            for jj in range(step):
                pair_fn(j0 + i * step + jj)
            return c
        with scope(f'pump_{pair_fn.__name__}_{j0}'):
            jax.lax.fori_loop(0, n // step, body, 0)

    start(x_hbm, x_vm, S_X, 0)
    start(gate_hbm, gate_vm, S_GATE, 0)
    pump_weights(160)

    sub = jax.lax.broadcasted_iota(jnp.int32, (8, D), 0)
    row = jax.lax.broadcasted_iota(jnp.int32, (H, D), 0)
    lane = jax.lax.broadcasted_iota(jnp.int32, (H, D), 1)
    diag = row == lane % H

    pltpu.make_async_copy(x_hbm, x_vm, sems.at[S_X]).wait()
    pltpu.make_async_copy(gate_hbm, gate_vm, sems.at[S_GATE]).wait()
    xf = x_vm[...].astype(F32)
    xf_vm[...] = xf
    start(xf_vm, x_smem, S_XS, 0)
    gw = gate_vm[...].astype(F32).reshape(1, M)
    z = jnp.sum(xf * gw, axis=-1, keepdims=True)
    g = 1.0 / (1.0 + jnp.exp(-z))

    wait_all(wqb_vm, S_WQB, 'wqb')
    if compute:
        x8 = jnp.broadcast_to(x_vm[...], (8, M))
        qb = jnp.dot(x8, wqb_vm[...], preferred_element_type=F32) * scale
        for h in range(H):
            qb_vm[h] = jnp.where(sub == h % 8, qb[:, h * D:(h + 1) * D], 0.0)
    pump_weights(80)

    pltpu.make_async_copy(xf_vm, x_smem, sems.at[S_XS]).wait()
    wait_all(wqa_vm, S_WQA, 'wqa')

    def qa_body(i, acc):
        for j in range(8):
            m = i * 8 + j
            acc = acc + wqa_vm[m].astype(F32) * x_smem[0, m]
        return acc

    if compute:
        with scope('qa'):
            qa = jax.lax.fori_loop(0, M // 8, qa_body, jnp.zeros((H, D), F32)).astype(BF16)
    pump_weights(64)

    wait_all(wuk_vm, S_WUK, 'wuk')

    def qlat_body(i, carry):
        rows8 = jnp.zeros((8, D), F32)
        for j in range(8):
            t = i * 8 + j
            w = jnp.concatenate([wuk_vm[cc * D + t] for cc in range(DC // D)], axis=0)
            prod = jax.lax.dot_general(qa, w, NT, preferred_element_type=F32)
            picked = jnp.sum(jnp.where(diag, prod, 0.0), axis=0, keepdims=True)
            rows8 = jnp.where(sub == j, picked, rows8)
        y_vm[pl.ds(pl.multiple_of(i * 8, 8), 8), :] = rows8
        for jj in range(3):
            pair_lead(wuv_hbm, wuv_vm, DC // 2, 4, 16 + i * 3 + jj, S_WUV)
        return carry

    if compute:
        with scope('qlat'):
            jax.lax.fori_loop(0, D // 8, qlat_body, 0)
        yt = y_vm[...].T
        qlat = jnp.concatenate([yt[cc * H:(cc + 1) * H, :] for cc in range(DC // D)], axis=1)
        qlat = (qlat * scale).astype(BF16)
    issued[0] += 48

    wait_all(ckv_vm, S_CKV, 'ckv')

    def score_body(i, mx):
        c = ckv_vm[pl.ds(pl.multiple_of(i * KB, KB), KB), :]
        s = jax.lax.dot_general(qlat, c, NT, preferred_element_type=F32)
        s_vm[i] = s
        for jj in range(4):
            pair_lead(woa_hbm, woa_vm, H * D // 2, WO_ROWS, i * 4 + jj, S_WOA)
        return jnp.maximum(mx, s)

    if compute:
        with scope('score'):
            mx = jax.lax.fori_loop(0, SK // KB, score_body, jnp.full((H, KB), -jnp.inf, F32))
        ma = jnp.max(mx, axis=-1, keepdims=True)
    issued[0] += 32

    def ctx_lat_body(i, carry):
        acc, lsum = carry
        p = jnp.exp(s_vm[i] - ma)
        c = ckv_vm[pl.ds(pl.multiple_of(i * KB, KB), KB), :]
        for jj in range(4):
            pair_lead(woa_hbm, woa_vm, H * D // 2, WO_ROWS, 32 + i * 4 + jj, S_WOA)
        return acc + jnp.dot(p.astype(BF16), c, preferred_element_type=F32), lsum + p

    if compute:
        with scope('ctxlat'):
            clat, lsum = jax.lax.fori_loop(
                0, SK // KB, ctx_lat_body, (jnp.zeros((H, DC), F32), jnp.zeros((H, KB), F32)))
        clat = clat / jnp.sum(lsum, axis=-1, keepdims=True)
    issued[0] += 32
    assert issued[0] == len(weight_pairs)

    wait_all(wuv_vm, S_WUV, 'wuv')
    if compute:
        u = jnp.concatenate([clat[:, cc * D:(cc + 1) * D] for cc in range(DC // D)], axis=0)
        y_vm[...] = u.T

    def ctx_body(i, acc):
        rows8 = y_vm[pl.ds(pl.multiple_of(i * 8, 8), 8), :]
        for j in range(8):
            t = i * 8 + j
            w = jnp.concatenate([wuv_vm[cc * D + t] for cc in range(DC // D)], axis=0)
            lhs = jnp.where(diag, jnp.broadcast_to(rows8[j:j + 1, :], (H, D)), 0.0)
            acc = acc + jnp.dot(lhs.astype(BF16), w, preferred_element_type=F32)
        for jj in range(3):
            pair_k(i * 3 + jj)
        return acc

    if compute:
        with scope('ctx'):
            ctx = jax.lax.fori_loop(0, D // 8, ctx_body, jnp.zeros((H, D), F32))
        for i in range(H // 8):
            ctx_vm[i] = ctx[i * 8:(i + 1) * 8, :]

    wait_all(woa_vm, S_WOA, 'woa')

    def proj_a_body(h, acc):
        lhs = jnp.where(sub == h % 8, ctx_vm[h // 8], 0.0)
        w = woa_vm[pl.ds(pl.multiple_of(h * D, D), D), :]
        for jj in range(2):
            pair_k(48 + h * 2 + jj)
        return acc + jnp.dot(lhs.astype(BF16), w, preferred_element_type=F32)

    if compute:
        with scope('proja'):
            a8 = jax.lax.fori_loop(0, H, proj_a_body, jnp.zeros((8, M), F32))
        ga = g * jnp.sum(a8, axis=0, keepdims=True)
    else:
        ga = jnp.zeros((1, M), F32)
    pump_loop(pair_k, 112, 224)

    def qk_group(g_idx, pair_fn, j0, n):
        wait_all(k_vm.at[pl.ds(g_idx * 8 * SK, 8 * SK)], K_SEM_OF_GROUP[g_idx], f'k{g_idx}')
        if compute:
            sb_vm[...] = jnp.zeros((8, SK), F32)

        def body(j, c):
            for jj in range(n):
                pair_fn(j0 + j * n + jj)
            if compute:
                h = g_idx * 8 + j
                kh = k_vm[pl.ds(pl.multiple_of(h * SK, SK), SK), :]
                sb_vm[...] += jax.lax.dot_general(qb_vm[h].astype(BF16), kh, NT,
                                                  preferred_element_type=F32)
            return c
        with scope(f'qk_{g_idx}'):
            jax.lax.fori_loop(0, 8, body, 0)
        if compute:
            s = sb_vm[...]
            p = jnp.exp(s - jnp.max(s, axis=-1, keepdims=True))
            l_vm[g_idx] = jnp.broadcast_to(jnp.sum(p, axis=-1, keepdims=True), (8, D))
            p_vm[g_idx] = p.astype(BF16)

    K_SEM_OF_GROUP = [S_K + 0, S_K + 1, S_K + 2, S_K + 3]
    qk_group(0, pair_k, 336, 11)
    qk_group(2, pair_k, 424, 11)
    pump_loop(pair_v, 0, 80)
    qk_group(1, pair_v, 80, 11)
    qk_group(3, pair_v, 168, 11)

    omg = 1.0 - g

    def pv_head(h):
        wait_all(v_vm.at[pl.ds(pl.multiple_of(h * SK, SK), SK)], S_V + h)
        if compute:
            vh = v_vm[pl.ds(pl.multiple_of(h * SK, SK), SK), :]
            o = jnp.dot(p_vm[h // 8], vh, preferred_element_type=F32)
            o = o * (omg / l_vm[h // 8])
            o = jnp.sum(jnp.where(sub == h % 8, o, 0.0), axis=0, keepdims=True)
            o_vm[h] = jnp.broadcast_to(o, (8, D))

    def pv_loop1(i, c):
        for jj in range(32):
            pair_v(256 + i * 32 + jj)
        pv_head(i)
        pv_head(16 + i)
        return c
    with scope('pv1'):
        jax.lax.fori_loop(0, 8, pv_loop1, 0)
    for i in range(8, 16):
        with scope(f'pv2_{i}'):
            for jj in range(8):
                pair_wob((i - 8) * 8 + jj)
            pv_head(i)
            pv_head(16 + i)

    vpu_units = cfg['vpu_units']
    n_mxu_units = len(b_units) - vpu_units
    b_starts = [H * D // 2]
    for rows in b_units:
        b_starts.append(b_starts[-1] + rows)
    vpu_row0 = b_starts[n_mxu_units]
    assert vpu_row0 % D == 0
    vpu_head0 = vpu_row0 // D
    if compute:
        for j in range(H - vpu_head0):
            ot_vm[pl.ds(j * D, D), :] = jnp.broadcast_to(o_vm[vpu_head0 + j][0:1, :], (D, D)).T
    b8 = jnp.zeros((8, M), F32)

    def proj_heads(b8, h0, h1):
        for h in range(h0, h1):
            b8 = b8 + jnp.dot(o_vm[h].astype(BF16), wob_vm[pl.ds(h * D, D), :],
                              preferred_element_type=F32)
        return b8

    wait_all(wob_vm.at[pl.ds(0, H * D // 2)], S_WOB, 'wobA')
    if compute:
        b8 = proj_heads(b8, 0, H // 2)
    for u in range(n_mxu_units):
        r0, n = b_starts[u], b_units[u]
        wait_all(wob_vm.at[pl.ds(r0, n)], S_WOB + 1 + u, f'wobB{u}')
        assert r0 % D == 0 and n % D == 0
        if compute:
            b8 = proj_heads(b8, r0 // D, (r0 + n) // D)
    out = ga + b8[0:1, :]
    for u in range(n_mxu_units, len(b_units)):
        s, n = b_starts[u], b_units[u]
        wait_all(wob_vm.at[pl.ds(s, n)], S_WOB + 1 + u, f'wobB{u}')
        if compute:
            w = wob_vm[pl.ds(s, n), :].astype(F32)
            o_col = ot_vm[pl.ds(s - vpu_row0, n), :]
            o_col = jnp.concatenate([o_col] * (M // D), axis=1)
            out = out + jnp.sum(w * o_col, axis=0, keepdims=True)
    out_ref[...] = out.astype(out_ref.dtype)


def make(compute=True, wob_b_units=(12 * 128, 2 * 128, 128, 96, 32), vpu_units=3, interpret=False, scopes=False):
    cfg = dict(scopes=scopes, compute=compute, wob_b_units=tuple(wob_b_units), vpu_units=vpu_units)
    vpu_rows = sum(wob_b_units[len(wob_b_units) - vpu_units:])

    def f(A_x, A_c_kv, A_w_q, A_w_uk, A_w_uv, A_w_o, B_x, B_k_cache, B_v_cache, B_wq, B_wo, gate_w):
        hbm = pl.BlockSpec(memory_space=pltpu.HBM)
        out = pl.pallas_call(
            functools.partial(_kernel, cfg=cfg),
            out_shape=jax.ShapeDtypeStruct((1, M), A_x.dtype),
            in_specs=[hbm] * 11,
            out_specs=pl.BlockSpec(memory_space=pltpu.VMEM),
            scratch_shapes=[
                pltpu.VMEM((1, M), BF16),
                pltpu.VMEM((M,), BF16),
                pltpu.VMEM((1, M), F32),
                pltpu.SMEM((1, M), F32),
                pltpu.VMEM((SK, DC), BF16),
                pltpu.VMEM((M, H, D), BF16),
                pltpu.VMEM((DC, H, D), BF16),
                pltpu.VMEM((DC, H, D), BF16),
                pltpu.VMEM((H * D, M), BF16),
                pltpu.VMEM((H * SK, D), BF16),
                pltpu.VMEM((H * SK, D), BF16),
                pltpu.VMEM((M, H * D), BF16),
                pltpu.VMEM((H * D, M), BF16),
                pltpu.VMEM((H, 8, D), F32),
                pltpu.VMEM((8, SK), F32),
                pltpu.VMEM((H // 8, 8, SK), BF16),
                pltpu.VMEM((H // 8, 8, D), F32),
                pltpu.VMEM((H, 8, D), F32),
                pltpu.VMEM((vpu_rows, D), F32),
                pltpu.VMEM((D, D), F32),
                pltpu.VMEM((SK // KB, H, KB), F32),
                pltpu.VMEM((H // 8, 8, D), F32),
            ],
            compiler_params=pltpu.CompilerParams(vmem_limit_bytes=112 << 20),
            interpret=interpret,
        )(
            A_x.reshape(1, M), gate_w,
            A_c_kv.reshape(SK, DC), A_w_q, A_w_uk, A_w_uv, A_w_o.reshape(H * D, M),
            B_k_cache.reshape(H * SK, D), B_v_cache.reshape(H * SK, D),
            B_wq, B_wo,
        )
        return out.reshape(1, 1, M)
    return f


_F = None


@jax.jit
def pallas_gated_mix__compressed_kv_cla__gqa_block_cached__decode_kernel(
    A_x, A_c_kv, A_w_q, A_w_uk, A_w_uv, A_w_o, B_x, B_k_cache, B_v_cache, B_wq, B_wo, gate_w,
):
    return make()(A_x, A_c_kv, A_w_q, A_w_uk, A_w_uv, A_w_o, B_x, B_k_cache, B_v_cache, B_wq, B_wo, gate_w)
```

```python
import contextlib
import functools

import jax
import jax.numpy as jnp
from jax.experimental import pallas as pl
from jax.experimental.pallas import tpu as pltpu

H = 32
D = 128
SK = 4096
M = 640
DC = 512
KB = 512
F32 = jnp.float32
BF16 = jnp.bfloat16
NT = (((1,), (1,)), ((), ()))

KV_ROWS = 128
WO_ROWS = 32
NS = 8

S_X, S_GATE, S_XS, S_WQB, S_WQA, S_WUK, S_CKV, S_WUV, S_WOA = range(9)
S_K = 9
S_V = S_K + 4
S_WOB = S_V + 4
S_TAIL = S_WOB + 3
N_SEMS = S_TAIL + 32


def _kernel(*refs, cfg):
    pl.run_scoped(functools.partial(_body, *refs, cfg=cfg), pltpu.SemaphoreType.DMA((N_SEMS,)))


def _body(x_hbm, gate_hbm, ckv_hbm, wqa_hbm, wuk_hbm, wuv_hbm, woa_hbm,
          k_hbm, v_hbm, wqb_hbm, wob_hbm,
          out_ref,
          x_vm, gate_vm, xf_vm, x_smem,
          ckv_vm, wqa_vm, wuk_vm, wuv_vm, woa_vm, k_vm, v_vm, wqb_vm, wob_vm,
          qb_vm, sb_vm, p_vm, l_vm, o_vm, ot_vm, y_vm, s_vm, ctx_vm, sems, *, cfg):
    scale = D ** -0.5

    def scope(name):
        return jax.named_scope(name) if cfg.get('scopes') else contextlib.nullcontext()

    def start(src, dst, sem, thread):
        pltpu.make_async_copy(src, dst, sems.at[sem]).start(thread)

    def wait_all(buf, sem, name=None):
        with (scope('wait_' + name) if name else contextlib.nullcontext()):
            pltpu.make_async_copy(buf, buf, sems.at[sem]).wait()

    def ds(off, n):
        return pl.ds(off if isinstance(off, int) else pl.multiple_of(off, n), n)

    def octet_w1(i):
        for q in range(4):
            idx = (ds(q * 160 + (i // 2) * 8, 8), ds((i % 2) * 2048, 2048))
            start(wqb_hbm.at[idx], wqb_vm.at[idx], S_WQB, 0)
            sl = ds(q * 160 + i * 4, 4)
            start(wqa_hbm.at[sl], wqa_vm.at[sl], S_WQA, 1)

    def octet_w2(i):
        for q in range(4):
            sl = ds(q * 128 + i * 4, 4)
            start(wuk_hbm.at[sl], wuk_vm.at[sl], S_WUK, 0)
            sl = ds(q * 1024 + i * 32, 32)
            start(ckv_hbm.at[sl], ckv_vm.at[sl], S_CKV, 1)

    def octet_w3(i):
        for q in range(4):
            sl = ds(q * 128 + i * 4, 4)
            start(wuv_hbm.at[sl], wuv_vm.at[sl], S_WUV, 0)
            sl = ds(q * 1024 + i * WO_ROWS, WO_ROWS)
            start(woa_hbm.at[sl], woa_vm.at[sl], S_WOA, 1)

    CPH = SK // KV_ROWS

    def octet_kv(hbm, vm, sem0, i):
        g, c = i // CPH, i % CPH
        for s in range(NS):
            src = ds((4 * s) * SK + i * KV_ROWS, KV_ROWS)
            dst = ds((g * 8 + s) * SK + c * KV_ROWS, KV_ROWS)
            start(hbm.at[src], vm.at[dst], sem0 + g, s % 2)

    octet_k = functools.partial(octet_kv, k_hbm, k_vm, S_K)
    octet_v = functools.partial(octet_kv, v_hbm, v_vm, S_V)

    def octet_wob(i):
        g, c = i // 4, i % 4
        for s in range(NS):
            src = pl.ds((4 * s + g) * D + c * WO_ROWS, WO_ROWS)
            dst = pl.ds((g * 8 + s) * D + c * WO_ROWS, WO_ROWS)
            sem = S_WOB + g if g < 3 else S_TAIL + s * 4 + c
            start(wob_hbm.at[src], wob_vm.at[dst], sem, s % 2)

    def octet_k_or_v(j):
        @pl.when(j < 128)
        def _():
            octet_k(j)

        @pl.when(j >= 128)
        def _():
            octet_v(j - 128)

    def pump(fn, i0, n, name):
        with scope('pump_' + name):
            if n % 2 == 0:
                def body(i, c):
                    fn(i0 + 2 * i)
                    fn(i0 + 2 * i + 1)
                    return c
                jax.lax.fori_loop(0, n // 2, body, 0)
            else:
                def body(i, c):
                    fn(i0 + i)
                    return c
                jax.lax.fori_loop(0, n, body, 0)

    start(x_hbm, x_vm, S_X, 0)
    start(gate_hbm, gate_vm, S_GATE, 0)
    pump(octet_w1, 0, 40, 'w1')
    pump(octet_w2, 0, 14, 'w2a')

    sub = jax.lax.broadcasted_iota(jnp.int32, (8, D), 0)
    row = jax.lax.broadcasted_iota(jnp.int32, (H, D), 0)
    lane = jax.lax.broadcasted_iota(jnp.int32, (H, D), 1)
    diag = row == lane % H

    pltpu.make_async_copy(x_hbm, x_vm, sems.at[S_X]).wait()
    pltpu.make_async_copy(gate_hbm, gate_vm, sems.at[S_GATE]).wait()
    xf = x_vm[...].astype(F32)
    xf_vm[...] = xf
    start(xf_vm, x_smem, S_XS, 0)
    gw = gate_vm[...].astype(F32).reshape(1, M)
    z = jnp.sum(xf * gw, axis=-1, keepdims=True)
    g = 1.0 / (1.0 + jnp.exp(-z))

    wait_all(wqb_vm, S_WQB, 'wqb')
    with scope('qb'):
        x8 = jnp.broadcast_to(x_vm[...], (8, M))
        qb = jnp.dot(x8, wqb_vm[...], preferred_element_type=F32) * scale
        for slot in range(H):
            h = 4 * (slot % 8) + slot // 8
            qb_vm[slot] = jnp.where(sub == slot % 8, qb[:, h * D:(h + 1) * D], 0.0)

    pltpu.make_async_copy(xf_vm, x_smem, sems.at[S_XS]).wait()
    wait_all(wqa_vm, S_WQA, 'wqa')

    def qa_outer(i, acc):
        octet_w2(14 + i)

        def qa_body(j, acc):
            for jj in range(8):
                m = i * 64 + j * 8 + jj
                acc = acc + wqa_vm[m].astype(F32) * x_smem[0, m]
            return acc
        return jax.lax.fori_loop(0, 8, qa_body, acc)

    with scope('qa'):
        qa = jax.lax.fori_loop(0, 10, qa_outer, jnp.zeros((H, D), F32)).astype(BF16)
    pump(octet_w2, 24, 8, 'w2b')
    pump(octet_w3, 0, 14, 'w3a')

    wait_all(wuk_vm, S_WUK, 'wuk')

    def qlat_body(i, carry):
        octet_w3(14 + i)
        rows8 = jnp.zeros((8, D), F32)
        for j in range(8):
            t = i * 8 + j
            w = jnp.concatenate([wuk_vm[cc * D + t] for cc in range(DC // D)], axis=0)
            prod = jax.lax.dot_general(qa, w, NT, preferred_element_type=F32)
            picked = jnp.sum(jnp.where(diag, prod, 0.0), axis=0, keepdims=True)
            rows8 = jnp.where(sub == j, picked, rows8)
        y_vm[pl.ds(pl.multiple_of(i * 8, 8), 8), :] = rows8
        return carry

    with scope('qlat'):
        jax.lax.fori_loop(0, D // 8, qlat_body, 0)
    octet_w3(30)
    octet_w3(31)
    yt = y_vm[...].T
    qlat = jnp.concatenate([yt[cc * H:(cc + 1) * H, :] for cc in range(DC // D)], axis=1)
    qlat = (qlat * scale).astype(BF16)

    wait_all(ckv_vm, S_CKV, 'ckv')

    def score_body(i, mx):
        octet_k(i)
        c = ckv_vm[pl.ds(pl.multiple_of(i * KB, KB), KB), :]
        s = jax.lax.dot_general(qlat, c, NT, preferred_element_type=F32)
        s_vm[i] = s
        return jnp.maximum(mx, s)

    with scope('score'):
        mx = jax.lax.fori_loop(0, SK // KB, score_body, jnp.full((H, KB), -jnp.inf, F32))
    ma = jnp.max(mx, axis=-1, keepdims=True)

    def ctx_lat_body(i, carry):
        octet_k(8 + i)
        acc, lsum = carry
        p = jnp.exp(s_vm[i] - ma)
        c = ckv_vm[pl.ds(pl.multiple_of(i * KB, KB), KB), :]
        return acc + jnp.dot(p.astype(BF16), c, preferred_element_type=F32), lsum + p

    with scope('ctxlat'):
        clat, lsum = jax.lax.fori_loop(
            0, SK // KB, ctx_lat_body, (jnp.zeros((H, DC), F32), jnp.zeros((H, KB), F32)))
    clat = clat / jnp.sum(lsum, axis=-1, keepdims=True)

    wait_all(wuv_vm, S_WUV, 'wuv')
    u = jnp.concatenate([clat[:, cc * D:(cc + 1) * D] for cc in range(DC // D)], axis=0)
    y_vm[...] = u.T

    def ctx_body(i, acc):
        octet_k(16 + i)
        rows8 = y_vm[pl.ds(pl.multiple_of(i * 8, 8), 8), :]
        for j in range(8):
            t = i * 8 + j
            w = jnp.concatenate([wuv_vm[cc * D + t] for cc in range(DC // D)], axis=0)
            lhs = jnp.where(diag, jnp.broadcast_to(rows8[j:j + 1, :], (H, D)), 0.0)
            acc = acc + jnp.dot(lhs.astype(BF16), w, preferred_element_type=F32)
        return acc

    with scope('ctx'):
        ctx = jax.lax.fori_loop(0, D // 8, ctx_body, jnp.zeros((H, D), F32))
    for i in range(H // 8):
        ctx_vm[i] = ctx[i * 8:(i + 1) * 8, :]

    wait_all(woa_vm, S_WOA, 'woa')

    def proj_a_body(i, acc):
        octet_k(32 + i)
        for jj in range(2):
            h = 2 * i + jj
            lhs = jnp.where(sub == h % 8, ctx_vm[h // 8], 0.0)
            w = woa_vm[pl.ds(pl.multiple_of(h * D, D), D), :]
            acc = acc + jnp.dot(lhs.astype(BF16), w, preferred_element_type=F32)
        return acc

    with scope('proja'):
        a8 = jax.lax.fori_loop(0, H // 2, proj_a_body, jnp.zeros((8, M), F32))
    ga = g * jnp.sum(a8, axis=0, keepdims=True)

    def qk_group(grp, j0):
        wait_all(k_vm.at[pl.ds(grp * 8 * SK, 8 * SK)], S_K + grp, f'k{grp}')
        sb_vm[...] = jnp.zeros((8, SK), F32)

        def body(j, c):
            for jj in range(4):
                octet_k_or_v(j0 + j * 4 + jj)
            slot = grp * 8 + j
            kh = k_vm[pl.ds(pl.multiple_of(slot * SK, SK), SK), :]
            sb_vm[...] += jax.lax.dot_general(qb_vm[slot].astype(BF16), kh, NT,
                                              preferred_element_type=F32)
            return c
        with scope(f'qk_{grp}'):
            jax.lax.fori_loop(0, 8, body, 0)
        s = sb_vm[...]
        p = jnp.exp(s - jnp.max(s, axis=-1, keepdims=True))
        l_vm[grp] = jnp.broadcast_to(jnp.sum(p, axis=-1, keepdims=True), (8, D))
        p_vm[grp] = p.astype(BF16)

    qk_group(0, 48)
    qk_group(1, 80)
    qk_group(2, 112)
    qk_group(3, 144)

    omg = 1.0 - g

    def pv_head(slot):
        grp = slot // 8
        vh = v_vm[pl.ds(pl.multiple_of(slot * SK, SK), SK), :]
        o = jnp.dot(p_vm[grp], vh, preferred_element_type=F32)
        o = o * (omg / l_vm[grp])
        o = jnp.sum(jnp.where(sub == slot % 8, o, 0.0), axis=0, keepdims=True)
        o_vm[slot] = jnp.broadcast_to(o, (8, D))

    def pv_group(grp, j0):
        wait_all(v_vm.at[pl.ds(grp * 8 * SK, 8 * SK)], S_V + grp, f'v{grp}')

        def body(j, c):
            if j0 is not None:
                for jj in range(4):
                    octet_v(j0 + j * 4 + jj)
            pv_head(grp * 8 + j)
            return c
        with scope(f'pv_{grp}'):
            jax.lax.fori_loop(0, 8, body, 0)

    pv_group(0, 48)
    pv_group(1, 80)
    wait_all(v_vm.at[pl.ds(2 * 8 * SK, 8 * SK)], S_V + 2, 'v2')
    with scope('pv_2'):
        for j in range(8):
            for jj in range(4):
                o_idx = 112 + j * 4 + jj
                if o_idx < 128:
                    octet_v(o_idx)
                else:
                    octet_wob(o_idx - 128)
            pv_head(16 + j)
    pv_group(3, None)

    for s in range(8):
        ot_vm[pl.ds(s * D, D), :] = jnp.broadcast_to(o_vm[24 + s][0:1, :], (D, D)).T
    b8 = jnp.zeros((8, M), F32)
    for grp in range(3):
        wait_all(wob_vm.at[pl.ds(grp * 8 * D, 8 * D)], S_WOB + grp, f'wob{grp}')
        for slot in range(grp * 8, grp * 8 + 8):
            b8 = b8 + jnp.dot(o_vm[slot].astype(BF16), wob_vm[pl.ds(slot * D, D), :],
                              preferred_element_type=F32)
    out = ga + b8[0:1, :]
    for c in range(4):
        for s in range(NS):
            r0 = (24 + s) * D + c * WO_ROWS
            src = wob_hbm.at[pl.ds((4 * s + 3) * D + c * WO_ROWS, WO_ROWS)]
            with scope(f'wait_tail{c}_{s}'):
                pltpu.make_async_copy(src, wob_vm.at[pl.ds(r0, WO_ROWS)], sems.at[S_TAIL + s * 4 + c]).wait()
            w = wob_vm[pl.ds(r0, WO_ROWS), :].astype(F32)
            o_col = ot_vm[pl.ds(s * D + c * WO_ROWS, WO_ROWS), :]
            o_col = jnp.concatenate([o_col] * (M // D), axis=1)
            out = out + jnp.sum(w * o_col, axis=0, keepdims=True)
    out_ref[...] = out.astype(out_ref.dtype)


def make(interpret=False, scopes=False):
    cfg = dict(scopes=scopes)

    def f(A_x, A_c_kv, A_w_q, A_w_uk, A_w_uv, A_w_o, B_x, B_k_cache, B_v_cache, B_wq, B_wo, gate_w):
        hbm = pl.BlockSpec(memory_space=pltpu.HBM)
        out = pl.pallas_call(
            functools.partial(_kernel, cfg=cfg),
            out_shape=jax.ShapeDtypeStruct((1, M), A_x.dtype),
            in_specs=[hbm] * 11,
            out_specs=pl.BlockSpec(memory_space=pltpu.VMEM),
            scratch_shapes=[
                pltpu.VMEM((1, M), BF16),
                pltpu.VMEM((M,), BF16),
                pltpu.VMEM((1, M), F32),
                pltpu.SMEM((1, M), F32),
                pltpu.VMEM((SK, DC), BF16),
                pltpu.VMEM((M, H, D), BF16),
                pltpu.VMEM((DC, H, D), BF16),
                pltpu.VMEM((DC, H, D), BF16),
                pltpu.VMEM((H * D, M), BF16),
                pltpu.VMEM((H * SK, D), BF16),
                pltpu.VMEM((H * SK, D), BF16),
                pltpu.VMEM((M, H * D), BF16),
                pltpu.VMEM((H * D, M), BF16),
                pltpu.VMEM((H, 8, D), F32),
                pltpu.VMEM((8, SK), F32),
                pltpu.VMEM((H // 8, 8, SK), BF16),
                pltpu.VMEM((H // 8, 8, D), F32),
                pltpu.VMEM((H, 8, D), F32),
                pltpu.VMEM((8 * D, D), F32),
                pltpu.VMEM((D, D), F32),
                pltpu.VMEM((SK // KB, H, KB), F32),
                pltpu.VMEM((H // 8, 8, D), F32),
            ],
            compiler_params=pltpu.CompilerParams(vmem_limit_bytes=112 << 20),
            interpret=interpret,
        )(
            A_x.reshape(1, M), gate_w,
            A_c_kv.reshape(SK, DC), A_w_q, A_w_uk, A_w_uv, A_w_o.reshape(H * D, M),
            B_k_cache.reshape(H * SK, D), B_v_cache.reshape(H * SK, D),
            B_wq, B_wo,
        )
        return out.reshape(1, 1, M)
    return f


_F = None


@jax.jit
def pallas_gated_mix__compressed_kv_cla__gqa_block_cached__decode_kernel(
    A_x, A_c_kv, A_w_q, A_w_uk, A_w_uv, A_w_o, B_x, B_k_cache, B_v_cache, B_wq, B_wo, gate_w,
):
    return make()(A_x, A_c_kv, A_w_q, A_w_uk, A_w_uv, A_w_o, B_x, B_k_cache, B_v_cache, B_wq, B_wo, gate_w)
```

```python
import contextlib
import functools

import jax
import jax.numpy as jnp
from jax.experimental import pallas as pl
from jax.experimental.pallas import tpu as pltpu

H = 32
D = 128
SK = 4096
M = 640
DC = 512
KB = 512
F32 = jnp.float32
BF16 = jnp.bfloat16
NT = (((1,), (1,)), ((), ()))

KV_ROWS = 128
WO_ROWS = 32
NS = 8

S_X, S_GATE, S_XS, S_WQB, S_WQA, S_WUK, S_CKV, S_WUV, S_WOA = range(9)
S_K = 9
S_V = S_K + 32
S_WOB = S_V + 32
S_TAIL = S_WOB + 3
N_SEMS = S_TAIL + 32


def _kernel(*refs, cfg):
    pl.run_scoped(functools.partial(_body, *refs, cfg=cfg), pltpu.SemaphoreType.DMA((N_SEMS,)))


def _body(x_hbm, gate_hbm, ckv_hbm, wqa_hbm, wuk_hbm, wuv_hbm, woa_hbm,
          k_hbm, v_hbm, wqb_hbm, wob_hbm,
          out_ref,
          x_vm, gate_vm, xf_vm, x_smem,
          ckv_vm, wqa_vm, wuk_vm, wuv_vm, woa_vm, k_vm, v_vm, wqb_vm, wob_vm,
          qb_vm, sb_vm, p_vm, l_vm, o_vm, ot_vm, y_vm, s_vm, ctx_vm, sems, *, cfg):
    scale = D ** -0.5

    def scope(name):
        return jax.named_scope(name) if cfg.get('scopes') else contextlib.nullcontext()

    def start(src, dst, sem, thread):
        pltpu.make_async_copy(src, dst, sems.at[sem]).start(thread)

    def wait_all(buf, sem, name=None):
        with (scope('wait_' + name) if name else contextlib.nullcontext()):
            pltpu.make_async_copy(buf, buf, sems.at[sem]).wait()

    def ds(off, n):
        return pl.ds(off if isinstance(off, int) else pl.multiple_of(off, n), n)

    def octet_w1(i):
        for q in range(4):
            idx = (ds(q * 160 + (i // 2) * 8, 8), ds((i % 2) * 2048, 2048))
            start(wqb_hbm.at[idx], wqb_vm.at[idx], S_WQB, 0)
            sl = ds(q * 160 + i * 4, 4)
            start(wqa_hbm.at[sl], wqa_vm.at[sl], S_WQA, 1)

    def octet_w2(i):
        for q in range(4):
            sl = ds(q * 128 + i * 4, 4)
            start(wuk_hbm.at[sl], wuk_vm.at[sl], S_WUK, 0)
            sl = ds(q * 1024 + i * 32, 32)
            start(ckv_hbm.at[sl], ckv_vm.at[sl], S_CKV, 1)

    def octet_w3(i):
        for q in range(4):
            sl = ds(q * 128 + i * 4, 4)
            start(wuv_hbm.at[sl], wuv_vm.at[sl], S_WUV, 0)
            sl = ds(q * 1024 + i * WO_ROWS, WO_ROWS)
            start(woa_hbm.at[sl], woa_vm.at[sl], S_WOA, 1)

    PH = cfg['phase']
    REG = 4 * SK
    NFULL = REG // KV_ROWS - (1 if PH else 0)

    def octet_full(hbm, vm, sem0, j):
        for s in range(NS):
            sl = pl.ds(pl.multiple_of(s * REG + PH + j * KV_ROWS, 8), KV_ROWS)
            start(hbm.at[sl], vm.at[sl], sem0 + s * 4 + j // 32, s % 2)

    def octet_first(hbm, vm, sem0):
        if PH:
            for s in range(NS):
                sl = pl.ds(s * REG, PH)
                start(hbm.at[sl], vm.at[sl], sem0 + s * 4, s % 2)

    def octet_last(hbm, vm, sem0):
        if PH:
            for s in range(NS):
                sl = pl.ds(s * REG + PH + NFULL * KV_ROWS, KV_ROWS - PH)
                start(hbm.at[sl], vm.at[sl], sem0 + s * 4 + 3, s % 2)

    def wait_group(vm, sem0, grp, name):
        r0 = 0 if grp == 0 else grp * SK + PH
        r1 = REG if grp == 3 else (grp + 1) * SK + PH
        with scope('wait_' + name):
            for s in range(NS):
                wait_all(vm.at[pl.ds(s * REG + r0, r1 - r0)], sem0 + s * 4 + grp)

    octet_k = functools.partial(octet_full, k_hbm, k_vm, S_K)
    octet_v = functools.partial(octet_full, v_hbm, v_vm, S_V)

    def octet_wob(i):
        g, c = i // 4, i % 4
        for s in range(NS):
            src = pl.ds((4 * s + g) * D + c * WO_ROWS, WO_ROWS)
            dst = pl.ds((g * 8 + s) * D + c * WO_ROWS, WO_ROWS)
            sem = S_WOB + g if g < 3 else S_TAIL + s * 4 + c
            start(wob_hbm.at[src], wob_vm.at[dst], sem, s % 2)

    def octet_k_or_v(u):
        @pl.when(u < NFULL)
        def _():
            octet_k(u)

        if PH:
            @pl.when(u == NFULL)
            def _():
                octet_last(k_hbm, k_vm, S_K)
                octet_first(v_hbm, v_vm, S_V)

        @pl.when(u >= 128)
        def _():
            octet_v(u - 128)

    def pump(fn, i0, n, name):
        with scope('pump_' + name):
            if n % 2 == 0:
                def body(i, c):
                    fn(i0 + 2 * i)
                    fn(i0 + 2 * i + 1)
                    return c
                jax.lax.fori_loop(0, n // 2, body, 0)
            else:
                def body(i, c):
                    fn(i0 + i)
                    return c
                jax.lax.fori_loop(0, n, body, 0)

    start(x_hbm, x_vm, S_X, 0)
    start(gate_hbm, gate_vm, S_GATE, 0)
    pump(octet_w1, 0, 40, 'w1')
    pump(octet_w2, 0, 14, 'w2a')

    sub = jax.lax.broadcasted_iota(jnp.int32, (8, D), 0)
    row = jax.lax.broadcasted_iota(jnp.int32, (H, D), 0)
    lane = jax.lax.broadcasted_iota(jnp.int32, (H, D), 1)
    diag = row == lane % H

    pltpu.make_async_copy(x_hbm, x_vm, sems.at[S_X]).wait()
    pltpu.make_async_copy(gate_hbm, gate_vm, sems.at[S_GATE]).wait()
    xf = x_vm[...].astype(F32)
    xf_vm[...] = xf
    start(xf_vm, x_smem, S_XS, 0)
    gw = gate_vm[...].astype(F32).reshape(1, M)
    z = jnp.sum(xf * gw, axis=-1, keepdims=True)
    g = 1.0 / (1.0 + jnp.exp(-z))

    wait_all(wqb_vm, S_WQB, 'wqb')
    with scope('qb'):
        x8 = jnp.broadcast_to(x_vm[...], (8, M))
        qb = jnp.dot(x8, wqb_vm[...], preferred_element_type=F32) * scale
        for slot in range(H):
            h = 4 * (slot % 8) + slot // 8
            qb_vm[slot] = jnp.where(sub == slot % 8, qb[:, h * D:(h + 1) * D], 0.0)

    pltpu.make_async_copy(xf_vm, x_smem, sems.at[S_XS]).wait()
    wait_all(wqa_vm, S_WQA, 'wqa')

    def qa_outer(i, acc):
        octet_w2(14 + i)

        def qa_body(j, acc):
            for jj in range(8):
                m = i * 64 + j * 8 + jj
                acc = acc + wqa_vm[m].astype(F32) * x_smem[0, m]
            return acc
        return jax.lax.fori_loop(0, 8, qa_body, acc)

    with scope('qa'):
        qa = jax.lax.fori_loop(0, 10, qa_outer, jnp.zeros((H, D), F32)).astype(BF16)
    pump(octet_w2, 24, 8, 'w2b')
    pump(octet_w3, 0, 14, 'w3a')

    wait_all(wuk_vm, S_WUK, 'wuk')

    def qlat_body(i, carry):
        octet_w3(14 + i)
        rows8 = jnp.zeros((8, D), F32)
        for j in range(8):
            t = i * 8 + j
            w = jnp.concatenate([wuk_vm[cc * D + t] for cc in range(DC // D)], axis=0)
            prod = jax.lax.dot_general(qa, w, NT, preferred_element_type=F32)
            picked = jnp.sum(jnp.where(diag, prod, 0.0), axis=0, keepdims=True)
            rows8 = jnp.where(sub == j, picked, rows8)
        y_vm[pl.ds(pl.multiple_of(i * 8, 8), 8), :] = rows8
        return carry

    with scope('qlat'):
        jax.lax.fori_loop(0, D // 8, qlat_body, 0)
    octet_w3(30)
    octet_w3(31)
    yt = y_vm[...].T
    qlat = jnp.concatenate([yt[cc * H:(cc + 1) * H, :] for cc in range(DC // D)], axis=1)
    qlat = (qlat * scale).astype(BF16)

    wait_all(ckv_vm, S_CKV, 'ckv')
    octet_first(k_hbm, k_vm, S_K)

    def score_body(i, mx):
        octet_k(i)
        c = ckv_vm[pl.ds(pl.multiple_of(i * KB, KB), KB), :]
        s = jax.lax.dot_general(qlat, c, NT, preferred_element_type=F32)
        s_vm[i] = s
        return jnp.maximum(mx, s)

    with scope('score'):
        mx = jax.lax.fori_loop(0, SK // KB, score_body, jnp.full((H, KB), -jnp.inf, F32))
    ma = jnp.max(mx, axis=-1, keepdims=True)

    def ctx_lat_body(i, carry):
        octet_k(8 + i)
        acc, lsum = carry
        p = jnp.exp(s_vm[i] - ma)
        c = ckv_vm[pl.ds(pl.multiple_of(i * KB, KB), KB), :]
        return acc + jnp.dot(p.astype(BF16), c, preferred_element_type=F32), lsum + p

    with scope('ctxlat'):
        clat, lsum = jax.lax.fori_loop(
            0, SK // KB, ctx_lat_body, (jnp.zeros((H, DC), F32), jnp.zeros((H, KB), F32)))
    clat = clat / jnp.sum(lsum, axis=-1, keepdims=True)

    wait_all(wuv_vm, S_WUV, 'wuv')
    u = jnp.concatenate([clat[:, cc * D:(cc + 1) * D] for cc in range(DC // D)], axis=0)
    y_vm[...] = u.T

    def ctx_body(i, acc):
        octet_k(16 + i)
        rows8 = y_vm[pl.ds(pl.multiple_of(i * 8, 8), 8), :]
        for j in range(8):
            t = i * 8 + j
            w = jnp.concatenate([wuv_vm[cc * D + t] for cc in range(DC // D)], axis=0)
            lhs = jnp.where(diag, jnp.broadcast_to(rows8[j:j + 1, :], (H, D)), 0.0)
            acc = acc + jnp.dot(lhs.astype(BF16), w, preferred_element_type=F32)
        return acc

    with scope('ctx'):
        ctx = jax.lax.fori_loop(0, D // 8, ctx_body, jnp.zeros((H, D), F32))
    for i in range(H // 8):
        ctx_vm[i] = ctx[i * 8:(i + 1) * 8, :]

    wait_all(woa_vm, S_WOA, 'woa')

    def proj_a_body(i, acc):
        octet_k(32 + i)
        for jj in range(2):
            h = 2 * i + jj
            lhs = jnp.where(sub == h % 8, ctx_vm[h // 8], 0.0)
            w = woa_vm[pl.ds(pl.multiple_of(h * D, D), D), :]
            acc = acc + jnp.dot(lhs.astype(BF16), w, preferred_element_type=F32)
        return acc

    with scope('proja'):
        a8 = jax.lax.fori_loop(0, H // 2, proj_a_body, jnp.zeros((8, M), F32))
    ga = g * jnp.sum(a8, axis=0, keepdims=True)

    def qk_group(grp, j0):
        wait_group(k_vm, S_K, grp, f'k{grp}')
        sb_vm[...] = jnp.zeros((8, SK), F32)

        def body(j, c):
            for jj in range(4):
                octet_k_or_v(j0 + j * 4 + jj)
            slot = grp * 8 + j
            kh = k_vm[pl.ds(pl.multiple_of((4 * j + grp) * SK, SK), SK), :]
            sb_vm[...] += jax.lax.dot_general(qb_vm[slot].astype(BF16), kh, NT,
                                              preferred_element_type=F32)
            return c
        with scope(f'qk_{grp}'):
            jax.lax.fori_loop(0, 8, body, 0)
        s = sb_vm[...]
        p = jnp.exp(s - jnp.max(s, axis=-1, keepdims=True))
        l_vm[grp] = jnp.broadcast_to(jnp.sum(p, axis=-1, keepdims=True), (8, D))
        p_vm[grp] = p.astype(BF16)

    qk_group(0, 48)
    qk_group(1, 80)
    qk_group(2, 112)
    qk_group(3, 144)

    omg = 1.0 - g

    def pv_head(slot):
        grp = slot // 8
        head = 4 * (slot % 8) + grp
        vh = v_vm[pl.ds(head * SK if isinstance(head, int) else pl.multiple_of(head * SK, SK), SK), :]
        o = jnp.dot(p_vm[grp], vh, preferred_element_type=F32)
        o = o * (omg / l_vm[grp])
        o = jnp.sum(jnp.where(sub == slot % 8, o, 0.0), axis=0, keepdims=True)
        o_vm[slot] = jnp.broadcast_to(o, (8, D))

    def pv_group(grp, j0):
        wait_group(v_vm, S_V, grp, f'v{grp}')

        def body(j, c):
            if j0 is not None:
                for jj in range(4):
                    octet_v(j0 + j * 4 + jj)
            pv_head(grp * 8 + j)
            return c
        with scope(f'pv_{grp}'):
            jax.lax.fori_loop(0, 8, body, 0)

    pv_group(0, 48)
    pv_group(1, 80)
    wait_group(v_vm, S_V, 2, 'v2')
    rest = [functools.partial(octet_v, j) for j in range(112, NFULL)]
    if PH:
        rest.append(functools.partial(octet_last, v_hbm, v_vm, S_V))
    rest += [functools.partial(octet_wob, i) for i in range(16)]
    assert len(rest) == 32
    with scope('pv_2'):
        for j in range(8):
            for fn in rest[4 * j:4 * j + 4]:
                fn()
            pv_head(16 + j)
    pv_group(3, None)

    for s in range(8):
        ot_vm[pl.ds(s * D, D), :] = jnp.broadcast_to(o_vm[24 + s][0:1, :], (D, D)).T
    b8 = jnp.zeros((8, M), F32)
    for grp in range(3):
        wait_all(wob_vm.at[pl.ds(grp * 8 * D, 8 * D)], S_WOB + grp, f'wob{grp}')
        for slot in range(grp * 8, grp * 8 + 8):
            b8 = b8 + jnp.dot(o_vm[slot].astype(BF16), wob_vm[pl.ds(slot * D, D), :],
                              preferred_element_type=F32)
    out = ga + b8[0:1, :]
    for c in range(4):
        for s in range(NS):
            r0 = (24 + s) * D + c * WO_ROWS
            src = wob_hbm.at[pl.ds((4 * s + 3) * D + c * WO_ROWS, WO_ROWS)]
            with scope(f'wait_tail{c}_{s}'):
                pltpu.make_async_copy(src, wob_vm.at[pl.ds(r0, WO_ROWS)], sems.at[S_TAIL + s * 4 + c]).wait()
            w = wob_vm[pl.ds(r0, WO_ROWS), :].astype(F32)
            o_col = ot_vm[pl.ds(s * D + c * WO_ROWS, WO_ROWS), :]
            o_col = jnp.concatenate([o_col] * (M // D), axis=1)
            out = out + jnp.sum(w * o_col, axis=0, keepdims=True)
    out_ref[...] = out.astype(out_ref.dtype)


def make(interpret=False, scopes=False, phase=64):
    cfg = dict(scopes=scopes, phase=phase)

    def f(A_x, A_c_kv, A_w_q, A_w_uk, A_w_uv, A_w_o, B_x, B_k_cache, B_v_cache, B_wq, B_wo, gate_w):
        hbm = pl.BlockSpec(memory_space=pltpu.HBM)
        out = pl.pallas_call(
            functools.partial(_kernel, cfg=cfg),
            out_shape=jax.ShapeDtypeStruct((1, M), A_x.dtype),
            in_specs=[hbm] * 11,
            out_specs=pl.BlockSpec(memory_space=pltpu.VMEM),
            scratch_shapes=[
                pltpu.VMEM((1, M), BF16),
                pltpu.VMEM((M,), BF16),
                pltpu.VMEM((1, M), F32),
                pltpu.SMEM((1, M), F32),
                pltpu.VMEM((SK, DC), BF16),
                pltpu.VMEM((M, H, D), BF16),
                pltpu.VMEM((DC, H, D), BF16),
                pltpu.VMEM((DC, H, D), BF16),
                pltpu.VMEM((H * D, M), BF16),
                pltpu.VMEM((H * SK, D), BF16),
                pltpu.VMEM((H * SK, D), BF16),
                pltpu.VMEM((M, H * D), BF16),
                pltpu.VMEM((H * D, M), BF16),
                pltpu.VMEM((H, 8, D), F32),
                pltpu.VMEM((8, SK), F32),
                pltpu.VMEM((H // 8, 8, SK), BF16),
                pltpu.VMEM((H // 8, 8, D), F32),
                pltpu.VMEM((H, 8, D), F32),
                pltpu.VMEM((8 * D, D), F32),
                pltpu.VMEM((D, D), F32),
                pltpu.VMEM((SK // KB, H, KB), F32),
                pltpu.VMEM((H // 8, 8, D), F32),
            ],
            compiler_params=pltpu.CompilerParams(vmem_limit_bytes=112 << 20),
            interpret=interpret,
        )(
            A_x.reshape(1, M), gate_w,
            A_c_kv.reshape(SK, DC), A_w_q, A_w_uk, A_w_uv, A_w_o.reshape(H * D, M),
            B_k_cache.reshape(H * SK, D), B_v_cache.reshape(H * SK, D),
            B_wq, B_wo,
        )
        return out.reshape(1, 1, M)
    return f


_F = None


@jax.jit
def pallas_gated_mix__compressed_kv_cla__gqa_block_cached__decode_kernel(
    A_x, A_c_kv, A_w_q, A_w_uk, A_w_uv, A_w_o, B_x, B_k_cache, B_v_cache, B_wq, B_wo, gate_w,
):
    return make()(A_x, A_c_kv, A_w_q, A_w_uk, A_w_uv, A_w_o, B_x, B_k_cache, B_v_cache, B_wq, B_wo, gate_w)
```

```python
import functools

import jax
import jax.numpy as jnp
from jax.experimental import pallas as pl
from jax.experimental.pallas import tpu as pltpu

H = 32
D = 128
SK = 4096
M = 640
DC = 512
KB = 512
F32 = jnp.float32
BF16 = jnp.bfloat16
NT = (((1,), (1,)), ((), ()))

NS = 8
KV_ROWS = 128
WO_ROWS = 32
REGION = 4 * SK
KV_LEAD = 64
KV_FULL = REGION // KV_ROWS - 1

VPU_GROUPS = (2, 3)
WO_AHEAD = 12

S_X, S_GATE, S_XS, S_WQB, S_WQA, S_WUK, S_CKV, S_WUV, S_WOA = range(9)
S_K = 9
S_V = S_K + 4 * NS
S_WOB = S_V + 4 * NS
S_TAIL = S_WOB + 2
N_SEMS = S_TAIL + len(VPU_GROUPS) * NS * (D // WO_ROWS)


def _kernel(*refs):
    pl.run_scoped(functools.partial(_body, *refs), pltpu.SemaphoreType.DMA((N_SEMS,)))


def _body(x_hbm, gate_hbm, ckv_hbm, wqa_hbm, wuk_hbm, wuv_hbm, woa_hbm,
          k_hbm, v_hbm, wqb_hbm, wob_hbm,
          out_ref,
          x_vm, gate_vm, xf_vm, x_smem,
          ckv_vm, wqa_vm, wuk_vm, wuv_vm, woa_vm, k_vm, v_vm, wqb_vm, wob_vm,
          qb_vm, sb_vm, p_vm, l_vm, o_vm, ot_vm, y_vm, s_vm, ctx_vm, sems):
    scale = D ** -0.5

    def start(src, dst, sem, thread):
        pltpu.make_async_copy(src, dst, sems.at[sem]).start(thread)

    def wait_all(buf, sem):
        pltpu.make_async_copy(buf, buf, sems.at[sem]).wait()

    def ds(start_, size, align):
        return pl.ds(start_ if isinstance(start_, int) else pl.multiple_of(start_, align), size)

    def octet_w1(i):
        for q in range(4):
            idx = (ds(q * 160 + (i // 2) * 8, 8, 8), ds((i % 2) * 2048, 2048, 2048))
            start(wqb_hbm.at[idx], wqb_vm.at[idx], S_WQB, 0)
            idx = ds(q * 160 + i * 4, 4, 4)
            start(wqa_hbm.at[idx], wqa_vm.at[idx], S_WQA, 1)

    def octet_w2(i):
        for q in range(4):
            idx = ds(q * 128 + i * 4, 4, 4)
            start(wuk_hbm.at[idx], wuk_vm.at[idx], S_WUK, 0)
            idx = ds(q * 1024 + i * 32, 32, 32)
            start(ckv_hbm.at[idx], ckv_vm.at[idx], S_CKV, 1)

    def octet_w3(i):
        for q in range(4):
            idx = ds(q * 128 + i * 4, 4, 4)
            start(wuv_hbm.at[idx], wuv_vm.at[idx], S_WUV, 0)
            idx = ds(q * 1024 + i * WO_ROWS, WO_ROWS, WO_ROWS)
            start(woa_hbm.at[idx], woa_vm.at[idx], S_WOA, 1)

    def octet_kv(hbm, vm, sem0, j):
        for s in range(NS):
            idx = ds(s * REGION + KV_LEAD + j * KV_ROWS, KV_ROWS, 8)
            start(hbm.at[idx], vm.at[idx], sem0 + 4 * s + j // (SK // KV_ROWS), s % 2)

    def octet_kv_lead(hbm, vm, sem0):
        for s in range(NS):
            idx = pl.ds(s * REGION, KV_LEAD)
            start(hbm.at[idx], vm.at[idx], sem0 + 4 * s, s % 2)

    def octet_kv_trail(hbm, vm, sem0):
        for s in range(NS):
            idx = pl.ds(s * REGION + KV_LEAD + KV_FULL * KV_ROWS, KV_ROWS - KV_LEAD)
            start(hbm.at[idx], vm.at[idx], sem0 + 4 * s + 3, s % 2)

    def wait_kv(vm, sem0, grp):
        r0 = 0 if grp == 0 else grp * SK + KV_LEAD
        r1 = REGION if grp == 3 else (grp + 1) * SK + KV_LEAD
        for s in range(NS):
            wait_all(vm.at[pl.ds(s * REGION + r0, r1 - r0)], sem0 + 4 * s + grp)

    octet_k = functools.partial(octet_kv, k_hbm, k_vm, S_K)
    octet_v = functools.partial(octet_kv, v_hbm, v_vm, S_V)

    def octet_k_then_v(u):
        @pl.when(u < KV_FULL)
        def _():
            octet_k(u)

        @pl.when(u == KV_FULL)
        def _():
            octet_kv_trail(k_hbm, k_vm, S_K)
            octet_kv_lead(v_hbm, v_vm, S_V)

        @pl.when(u > KV_FULL)
        def _():
            octet_v(u - KV_FULL - 1)

    def wob_copy(grp, s, c):
        src = wob_hbm.at[pl.ds((4 * s + grp) * D + c * WO_ROWS, WO_ROWS)]
        dst = wob_vm.at[pl.ds((grp * 8 + s) * D + c * WO_ROWS, WO_ROWS)]
        if grp in VPU_GROUPS:
            sem = S_TAIL + (VPU_GROUPS.index(grp) * NS + s) * (D // WO_ROWS) + c
        else:
            sem = S_WOB + grp
        return pltpu.make_async_copy(src, dst, sems.at[sem])

    def octet_wob(i):
        for s in range(NS):
            wob_copy(i // (D // WO_ROWS), s, i % (D // WO_ROWS)).start(s % 2)

    def pump(octet, first, count):
        def body(i, carry):
            octet(first + 2 * i)
            octet(first + 2 * i + 1)
            return carry
        jax.lax.fori_loop(0, count // 2, body, 0)

    sub = jax.lax.broadcasted_iota(jnp.int32, (8, D), 0)
    row = jax.lax.broadcasted_iota(jnp.int32, (H, D), 0)
    lane = jax.lax.broadcasted_iota(jnp.int32, (H, D), 1)
    diag = row == lane % H

    start(x_hbm, x_vm, S_X, 0)
    start(gate_hbm, gate_vm, S_GATE, 0)
    pump(octet_w1, 0, 40)
    pump(octet_w2, 0, 14)

    pltpu.make_async_copy(x_hbm, x_vm, sems.at[S_X]).wait()
    pltpu.make_async_copy(gate_hbm, gate_vm, sems.at[S_GATE]).wait()
    xf = x_vm[...].astype(F32)
    xf_vm[...] = xf
    x_to_smem = pltpu.make_async_copy(xf_vm, x_smem, sems.at[S_XS])
    x_to_smem.start()
    gw = gate_vm[...].astype(F32).reshape(1, M)
    z = jnp.sum(xf * gw, axis=-1, keepdims=True)
    g = 1.0 / (1.0 + jnp.exp(-z))

    wait_all(wqb_vm, S_WQB)
    x8 = jnp.broadcast_to(x_vm[...], (8, M))
    qb = jnp.dot(x8, wqb_vm[...], preferred_element_type=F32) * scale
    for slot in range(H):
        h = 4 * (slot % 8) + slot // 8
        qb_vm[slot] = jnp.where(sub == slot % 8, qb[:, h * D:(h + 1) * D], 0.0)

    x_to_smem.wait()
    wait_all(wqa_vm, S_WQA)

    def qa_outer(i, acc):
        octet_w2(14 + i)

        def qa_inner(j, acc):
            for jj in range(8):
                m = i * 64 + j * 8 + jj
                acc = acc + wqa_vm[m].astype(F32) * x_smem[0, m]
            return acc

        return jax.lax.fori_loop(0, 8, qa_inner, acc)

    qa = jax.lax.fori_loop(0, M // 64, qa_outer, jnp.zeros((H, D), F32)).astype(BF16)
    pump(octet_w2, 24, 8)
    pump(octet_w3, 0, 14)

    wait_all(wuk_vm, S_WUK)

    def qlat_body(i, carry):
        octet_w3(14 + i)
        rows8 = jnp.zeros((8, D), F32)
        for j in range(8):
            t = i * 8 + j
            w = jnp.concatenate([wuk_vm[cc * D + t] for cc in range(DC // D)], axis=0)
            prod = jax.lax.dot_general(qa, w, NT, preferred_element_type=F32)
            picked = jnp.sum(jnp.where(diag, prod, 0.0), axis=0, keepdims=True)
            rows8 = jnp.where(sub == j, picked, rows8)
        y_vm[pl.ds(pl.multiple_of(i * 8, 8), 8), :] = rows8
        return carry

    jax.lax.fori_loop(0, D // 8, qlat_body, 0)
    octet_w3(30)
    octet_w3(31)
    yt = y_vm[...].T
    qlat = jnp.concatenate([yt[cc * H:(cc + 1) * H, :] for cc in range(DC // D)], axis=1)
    qlat = (qlat * scale).astype(BF16)

    wait_all(ckv_vm, S_CKV)
    octet_kv_lead(k_hbm, k_vm, S_K)

    def score_body(i, mx):
        octet_k(i)
        c = ckv_vm[pl.ds(pl.multiple_of(i * KB, KB), KB), :]
        s = jax.lax.dot_general(qlat, c, NT, preferred_element_type=F32)
        s_vm[i] = s
        return jnp.maximum(mx, s)

    mx = jax.lax.fori_loop(0, SK // KB, score_body, jnp.full((H, KB), -jnp.inf, F32))
    ma = jnp.max(mx, axis=-1, keepdims=True)

    def ctx_lat_body(i, carry):
        octet_k(8 + i)
        acc, lsum = carry
        p = jnp.exp(s_vm[i] - ma)
        c = ckv_vm[pl.ds(pl.multiple_of(i * KB, KB), KB), :]
        return acc + jnp.dot(p.astype(BF16), c, preferred_element_type=F32), lsum + p

    clat, lsum = jax.lax.fori_loop(
        0, SK // KB, ctx_lat_body, (jnp.zeros((H, DC), F32), jnp.zeros((H, KB), F32)))
    clat = clat / jnp.sum(lsum, axis=-1, keepdims=True)

    wait_all(wuv_vm, S_WUV)
    u = jnp.concatenate([clat[:, cc * D:(cc + 1) * D] for cc in range(DC // D)], axis=0)
    y_vm[...] = u.T

    def ctx_body(i, acc):
        octet_k(16 + i)
        rows8 = y_vm[pl.ds(pl.multiple_of(i * 8, 8), 8), :]
        for j in range(8):
            t = i * 8 + j
            w = jnp.concatenate([wuv_vm[cc * D + t] for cc in range(DC // D)], axis=0)
            lhs = jnp.where(diag, jnp.broadcast_to(rows8[j:j + 1, :], (H, D)), 0.0)
            acc = acc + jnp.dot(lhs.astype(BF16), w, preferred_element_type=F32)
        return acc

    ctx = jax.lax.fori_loop(0, D // 8, ctx_body, jnp.zeros((H, D), F32))
    for i in range(H // 8):
        ctx_vm[i] = ctx[i * 8:(i + 1) * 8, :]

    wait_all(woa_vm, S_WOA)

    def proj_a_body(i, acc):
        octet_k(32 + i)
        for jj in range(2):
            h = 2 * i + jj
            lhs = jnp.where(sub == h % 8, ctx_vm[h // 8], 0.0)
            w = woa_vm[pl.ds(pl.multiple_of(h * D, D), D), :]
            acc = acc + jnp.dot(lhs.astype(BF16), w, preferred_element_type=F32)
        return acc

    a8 = jax.lax.fori_loop(0, H // 2, proj_a_body, jnp.zeros((8, M), F32))
    ga = g * jnp.sum(a8, axis=0, keepdims=True)

    def softmax_b(grp, first_octet):
        wait_kv(k_vm, S_K, grp)
        sb_vm[...] = jnp.zeros((8, SK), F32)

        def body(s, carry):
            for jj in range(4):
                octet_k_then_v(first_octet + s * 4 + jj)
            kh = k_vm[pl.ds(pl.multiple_of((4 * s + grp) * SK, SK), SK), :]
            sb_vm[...] += jax.lax.dot_general(qb_vm[grp * 8 + s].astype(BF16), kh, NT,
                                              preferred_element_type=F32)
            return carry

        jax.lax.fori_loop(0, 8, body, 0)
        sc = sb_vm[...]
        p = jnp.exp(sc - jnp.max(sc, axis=-1, keepdims=True))
        l_vm[grp] = jnp.broadcast_to(jnp.sum(p, axis=-1, keepdims=True), (8, D))
        p_vm[grp] = p.astype(BF16)

    for grp in range(4):
        softmax_b(grp, 48 + 32 * grp)

    omg = 1.0 - g

    def pv_head(grp, s):
        vh = v_vm[ds((4 * s + grp) * SK, SK, SK), :]
        o = jnp.dot(p_vm[grp], vh, preferred_element_type=F32)
        o = o * (omg / l_vm[grp])
        o = jnp.sum(jnp.where(sub == s, o, 0.0), axis=0, keepdims=True)
        o_vm[grp * 8 + s] = jnp.broadcast_to(o, (8, D))

    def pv_group(grp, first_octet):
        wait_kv(v_vm, S_V, grp)

        def body(s, carry):
            for jj in range(4):
                octet_v(first_octet + s * 4 + jj)
            pv_head(grp, s)
            return carry

        jax.lax.fori_loop(0, 8, body, 0)

    def columns(grp):
        base = VPU_GROUPS.index(grp) * 8 * D
        for s in range(8):
            ot_vm[pl.ds(base + s * D, D), :] = jnp.broadcast_to(o_vm[grp * 8 + s][0:1, :], (D, D)).T

    pv_group(0, 48)
    pv_group(1, 80)
    wait_kv(v_vm, S_V, 2)
    v_rest = [functools.partial(octet_v, j) for j in range(112, KV_FULL)]
    v_rest.append(functools.partial(octet_kv_trail, v_hbm, v_vm, S_V))
    for s in range(8):
        for octet in v_rest[2 * s:2 * s + 2]:
            octet()
        pv_head(2, s)
    columns(2)
    for i in range(WO_AHEAD):
        octet_wob(i)
    wait_kv(v_vm, S_V, 3)
    for s in range(8):
        if WO_AHEAD + s < 16:
            octet_wob(WO_AHEAD + s)
        pv_head(3, s)
    columns(3)

    b8 = jnp.zeros((8, M), F32)
    for grp in range(4):
        if grp not in VPU_GROUPS:
            wait_all(wob_vm.at[pl.ds(grp * 8 * D, 8 * D)], S_WOB + grp)
            for slot in range(grp * 8, grp * 8 + 8):
                b8 = b8 + jnp.dot(o_vm[slot].astype(BF16), wob_vm[pl.ds(slot * D, D), :],
                                  preferred_element_type=F32)
    out = ga + b8[0:1, :]
    for grp in VPU_GROUPS:
        for c in range(D // WO_ROWS):
            for s in range(NS):
                wob_copy(grp, s, c).wait()
                w = wob_vm[pl.ds((grp * 8 + s) * D + c * WO_ROWS, WO_ROWS), :].astype(F32)
                r0 = (VPU_GROUPS.index(grp) * 8 + s) * D + c * WO_ROWS
                o_col = jnp.concatenate([ot_vm[pl.ds(r0, WO_ROWS), :]] * (M // D), axis=1)
                out = out + jnp.sum(w * o_col, axis=0, keepdims=True)
    out_ref[...] = out.astype(out_ref.dtype)


def _forward(A_x, A_c_kv, A_w_q, A_w_uk, A_w_uv, A_w_o, B_k_cache, B_v_cache, B_wq, B_wo,
             gate_w, interpret=False):
    hbm = pl.BlockSpec(memory_space=pltpu.HBM)
    out = pl.pallas_call(
        _kernel,
        out_shape=jax.ShapeDtypeStruct((1, M), A_x.dtype),
        in_specs=[hbm] * 11,
        out_specs=pl.BlockSpec(memory_space=pltpu.VMEM),
        scratch_shapes=[
            pltpu.VMEM((1, M), BF16),
            pltpu.VMEM((M,), BF16),
            pltpu.VMEM((1, M), F32),
            pltpu.SMEM((1, M), F32),
            pltpu.VMEM((SK, DC), BF16),
            pltpu.VMEM((M, H, D), BF16),
            pltpu.VMEM((DC, H, D), BF16),
            pltpu.VMEM((DC, H, D), BF16),
            pltpu.VMEM((H * D, M), BF16),
            pltpu.VMEM((H * SK, D), BF16),
            pltpu.VMEM((H * SK, D), BF16),
            pltpu.VMEM((M, H * D), BF16),
            pltpu.VMEM((H * D, M), BF16),
            pltpu.VMEM((H, 8, D), F32),
            pltpu.VMEM((8, SK), F32),
            pltpu.VMEM((H // 8, 8, SK), BF16),
            pltpu.VMEM((H // 8, 8, D), F32),
            pltpu.VMEM((H, 8, D), F32),
            pltpu.VMEM((len(VPU_GROUPS) * 8 * D, D), F32),
            pltpu.VMEM((D, D), F32),
            pltpu.VMEM((SK // KB, H, KB), F32),
            pltpu.VMEM((H // 8, 8, D), F32),
        ],
        compiler_params=pltpu.CompilerParams(vmem_limit_bytes=112 << 20),
        interpret=interpret,
    )(
        A_x.reshape(1, M), gate_w,
        A_c_kv.reshape(SK, DC), A_w_q, A_w_uk, A_w_uv, A_w_o.reshape(H * D, M),
        B_k_cache.reshape(H * SK, D), B_v_cache.reshape(H * SK, D),
        B_wq, B_wo,
    )
    return out.reshape(1, 1, M)


@jax.jit
def pallas_gated_mix__compressed_kv_cla__gqa_block_cached__decode_kernel(
    A_x: jax.Array,
    A_c_kv: jax.Array,
    A_w_q: jax.Array,
    A_w_uk: jax.Array,
    A_w_uv: jax.Array,
    A_w_o: jax.Array,
    B_x: jax.Array,
    B_k_cache: jax.Array,
    B_v_cache: jax.Array,
    B_wq: jax.Array,
    B_wo: jax.Array,
    gate_w: jax.Array,
):
    del B_x
    return _forward(A_x, A_c_kv, A_w_q, A_w_uk, A_w_uv, A_w_o,
                    B_k_cache, B_v_cache, B_wq, B_wo, gate_w)
```

```python
import functools

import jax
import jax.numpy as jnp
from jax.experimental import pallas as pl
from jax.experimental.pallas import tpu as pltpu

H = 32
D = 128
SK = 4096
M = 640
DC = 512
KB = 512
F32 = jnp.float32
BF16 = jnp.bfloat16
NT = (((1,), (1,)), ((), ()))

NS = 8
KV_ROWS = 128
WO_ROWS = 32
REGION = 4 * SK
KV_LEAD = 64
KV_FULL = REGION // KV_ROWS - 1

VPU_GROUPS = (2, 3)
WO_AHEAD = 12

S_X, S_GATE, S_XS, S_WQB, S_WQA, S_WUK, S_CKV, S_WUV, S_WOA = range(9)
S_K = 9
S_V = S_K + 4 * NS
S_WOB = S_V + 4 * NS
S_TAIL = S_WOB + 2
N_SEMS = S_TAIL + len(VPU_GROUPS) * NS * (D // WO_ROWS)


def _kernel(*refs):
    pl.run_scoped(functools.partial(_body, *refs), pltpu.SemaphoreType.DMA((N_SEMS,)))


def _body(x_hbm, gate_hbm, ckv_hbm, wqa_hbm, wuk_hbm, wuv_hbm, woa_hbm,
          k_hbm, v_hbm, wqb_hbm, wob_hbm,
          out_ref,
          x_vm, gate_vm, xf_vm, x_smem,
          ckv_vm, wqa_vm, wuk_vm, wuv_vm, woa_vm, k_vm, v_vm, wqb_vm, wob_vm,
          qb_vm, sb_vm, p_vm, l_vm, o_vm, ot_vm, y_vm, s_vm, ctx_vm, sems):
    scale = D ** -0.5

    def start(src, dst, sem, thread):
        pltpu.make_async_copy(src, dst, sems.at[sem]).start(thread)

    def wait_all(buf, sem):
        pltpu.make_async_copy(buf, buf, sems.at[sem]).wait()

    def ds(start_, size, align):
        return pl.ds(start_ if isinstance(start_, int) else pl.multiple_of(start_, align), size)

    def wqb_piece(q, strip, col0, cols):
        idx = (ds(q * 160 + strip * 8, 8, 8), pl.ds(col0, cols))
        start(wqb_hbm.at[idx], wqb_vm.at[idx], S_WQB, 0)

    def wqa_piece(q, i):
        idx = ds(q * 160 + i * 4, 4, 4)
        start(wqa_hbm.at[idx], wqa_vm.at[idx], S_WQA, 1)

    def w1_lead():
        for q in range(4):
            wqb_piece(q, 0, 0, 1024)

    def w1_strip(r):
        for q in range(4):
            wqb_piece(q, r, 1024, 2048)
            wqa_piece(q, 2 * r)
        for q in range(4):
            wqb_piece(q, r, 3072, 1024)
            wqa_piece(q, 2 * r + 1)

        @pl.when(r + 1 < 20)
        def _():
            for q in range(4):
                wqb_piece(q, r + 1, 0, 1024)

    def octet_w2(i):
        for q in range(4):
            idx = ds(q * 128 + i * 4, 4, 4)
            start(wuk_hbm.at[idx], wuk_vm.at[idx], S_WUK, 0)
            idx = ds(q * 1024 + i * 32, 32, 32)
            start(ckv_hbm.at[idx], ckv_vm.at[idx], S_CKV, 1)

    def octet_w3(i):
        for q in range(4):
            idx = ds(q * 128 + i * 4, 4, 4)
            start(wuv_hbm.at[idx], wuv_vm.at[idx], S_WUV, 0)
            idx = ds(q * 1024 + i * WO_ROWS, WO_ROWS, WO_ROWS)
            start(woa_hbm.at[idx], woa_vm.at[idx], S_WOA, 1)

    def octet_kv(hbm, vm, sem0, j):
        for s in range(NS):
            idx = ds(s * REGION + KV_LEAD + j * KV_ROWS, KV_ROWS, 8)
            start(hbm.at[idx], vm.at[idx], sem0 + 4 * s + j // (SK // KV_ROWS), s % 2)

    def octet_kv_lead(hbm, vm, sem0):
        for s in range(NS):
            idx = pl.ds(s * REGION, KV_LEAD)
            start(hbm.at[idx], vm.at[idx], sem0 + 4 * s, s % 2)

    def octet_kv_trail(hbm, vm, sem0):
        for s in range(NS):
            idx = pl.ds(s * REGION + KV_LEAD + KV_FULL * KV_ROWS, KV_ROWS - KV_LEAD)
            start(hbm.at[idx], vm.at[idx], sem0 + 4 * s + 3, s % 2)

    def wait_kv(vm, sem0, grp):
        r0 = 0 if grp == 0 else grp * SK + KV_LEAD
        r1 = REGION if grp == 3 else (grp + 1) * SK + KV_LEAD
        for s in range(NS):
            wait_all(vm.at[pl.ds(s * REGION + r0, r1 - r0)], sem0 + 4 * s + grp)

    octet_k = functools.partial(octet_kv, k_hbm, k_vm, S_K)
    octet_v = functools.partial(octet_kv, v_hbm, v_vm, S_V)

    def octet_k_then_v(u):
        @pl.when(u < KV_FULL)
        def _():
            octet_k(u)

        @pl.when(u == KV_FULL)
        def _():
            octet_kv_trail(k_hbm, k_vm, S_K)
            octet_kv_lead(v_hbm, v_vm, S_V)

        @pl.when(u > KV_FULL)
        def _():
            octet_v(u - KV_FULL - 1)

    def wob_copy(grp, s, c):
        src = wob_hbm.at[pl.ds((4 * s + grp) * D + c * WO_ROWS, WO_ROWS)]
        dst = wob_vm.at[pl.ds((grp * 8 + s) * D + c * WO_ROWS, WO_ROWS)]
        if grp in VPU_GROUPS:
            sem = S_TAIL + (VPU_GROUPS.index(grp) * NS + s) * (D // WO_ROWS) + c
        else:
            sem = S_WOB + grp
        return pltpu.make_async_copy(src, dst, sems.at[sem])

    def octet_wob(i):
        for s in range(NS):
            wob_copy(i // (D // WO_ROWS), s, i % (D // WO_ROWS)).start(s % 2)

    def pump(octet, first, count):
        def body(i, carry):
            octet(first + 2 * i)
            octet(first + 2 * i + 1)
            return carry
        jax.lax.fori_loop(0, count // 2, body, 0)

    sub = jax.lax.broadcasted_iota(jnp.int32, (8, D), 0)
    row = jax.lax.broadcasted_iota(jnp.int32, (H, D), 0)
    lane = jax.lax.broadcasted_iota(jnp.int32, (H, D), 1)
    diag = row == lane % H

    start(x_hbm, x_vm, S_X, 0)
    start(gate_hbm, gate_vm, S_GATE, 0)
    w1_lead()
    jax.lax.fori_loop(0, 20, lambda r, carry: (w1_strip(r), carry)[1], 0)
    pump(octet_w2, 0, 14)

    pltpu.make_async_copy(x_hbm, x_vm, sems.at[S_X]).wait()
    pltpu.make_async_copy(gate_hbm, gate_vm, sems.at[S_GATE]).wait()
    xf = x_vm[...].astype(F32)
    xf_vm[...] = xf
    x_to_smem = pltpu.make_async_copy(xf_vm, x_smem, sems.at[S_XS])
    x_to_smem.start()
    gw = gate_vm[...].astype(F32).reshape(1, M)
    z = jnp.sum(xf * gw, axis=-1, keepdims=True)
    g = 1.0 / (1.0 + jnp.exp(-z))

    wait_all(wqb_vm, S_WQB)
    x8 = jnp.broadcast_to(x_vm[...], (8, M))
    qb = jnp.dot(x8, wqb_vm[...], preferred_element_type=F32) * scale
    for slot in range(H):
        h = 4 * (slot % 8) + slot // 8
        qb_vm[slot] = jnp.where(sub == slot % 8, qb[:, h * D:(h + 1) * D], 0.0)

    x_to_smem.wait()
    wait_all(wqa_vm, S_WQA)

    def qa_outer(i, acc):
        octet_w2(14 + i)

        def qa_inner(j, acc):
            for jj in range(8):
                m = i * 64 + j * 8 + jj
                acc = acc + wqa_vm[m].astype(F32) * x_smem[0, m]
            return acc

        return jax.lax.fori_loop(0, 8, qa_inner, acc)

    qa = jax.lax.fori_loop(0, M // 64, qa_outer, jnp.zeros((H, D), F32)).astype(BF16)
    pump(octet_w2, 24, 8)
    pump(octet_w3, 0, 14)

    wait_all(wuk_vm, S_WUK)

    def qlat_body(i, carry):
        octet_w3(14 + i)
        rows8 = jnp.zeros((8, D), F32)
        for j in range(8):
            t = i * 8 + j
            w = jnp.concatenate([wuk_vm[cc * D + t] for cc in range(DC // D)], axis=0)
            prod = jax.lax.dot_general(qa, w, NT, preferred_element_type=F32)
            picked = jnp.sum(jnp.where(diag, prod, 0.0), axis=0, keepdims=True)
            rows8 = jnp.where(sub == j, picked, rows8)
        y_vm[pl.ds(pl.multiple_of(i * 8, 8), 8), :] = rows8
        return carry

    jax.lax.fori_loop(0, D // 8, qlat_body, 0)
    octet_w3(30)
    octet_w3(31)
    yt = y_vm[...].T
    qlat = jnp.concatenate([yt[cc * H:(cc + 1) * H, :] for cc in range(DC // D)], axis=1)
    qlat = (qlat * scale).astype(BF16)

    wait_all(ckv_vm, S_CKV)
    octet_kv_lead(k_hbm, k_vm, S_K)

    def score_body(i, mx):
        octet_k(i)
        c = ckv_vm[pl.ds(pl.multiple_of(i * KB, KB), KB), :]
        s = jax.lax.dot_general(qlat, c, NT, preferred_element_type=F32)
        s_vm[i] = s
        return jnp.maximum(mx, s)

    mx = jax.lax.fori_loop(0, SK // KB, score_body, jnp.full((H, KB), -jnp.inf, F32))
    ma = jnp.max(mx, axis=-1, keepdims=True)

    def ctx_lat_body(i, carry):
        octet_k(8 + i)
        acc, lsum = carry
        p = jnp.exp(s_vm[i] - ma)
        c = ckv_vm[pl.ds(pl.multiple_of(i * KB, KB), KB), :]
        return acc + jnp.dot(p.astype(BF16), c, preferred_element_type=F32), lsum + p

    clat, lsum = jax.lax.fori_loop(
        0, SK // KB, ctx_lat_body, (jnp.zeros((H, DC), F32), jnp.zeros((H, KB), F32)))
    clat = clat / jnp.sum(lsum, axis=-1, keepdims=True)

    wait_all(wuv_vm, S_WUV)
    u = jnp.concatenate([clat[:, cc * D:(cc + 1) * D] for cc in range(DC // D)], axis=0)
    y_vm[...] = u.T

    def ctx_body(i, acc):
        octet_k(16 + i)
        rows8 = y_vm[pl.ds(pl.multiple_of(i * 8, 8), 8), :]
        for j in range(8):
            t = i * 8 + j
            w = jnp.concatenate([wuv_vm[cc * D + t] for cc in range(DC // D)], axis=0)
            lhs = jnp.where(diag, jnp.broadcast_to(rows8[j:j + 1, :], (H, D)), 0.0)
            acc = acc + jnp.dot(lhs.astype(BF16), w, preferred_element_type=F32)
        return acc

    ctx = jax.lax.fori_loop(0, D // 8, ctx_body, jnp.zeros((H, D), F32))
    for i in range(H // 8):
        ctx_vm[i] = ctx[i * 8:(i + 1) * 8, :]

    wait_all(woa_vm, S_WOA)

    def proj_a_body(i, acc):
        octet_k(32 + i)
        for jj in range(2):
            h = 2 * i + jj
            lhs = jnp.where(sub == h % 8, ctx_vm[h // 8], 0.0)
            w = woa_vm[pl.ds(pl.multiple_of(h * D, D), D), :]
            acc = acc + jnp.dot(lhs.astype(BF16), w, preferred_element_type=F32)
        return acc

    a8 = jax.lax.fori_loop(0, H // 2, proj_a_body, jnp.zeros((8, M), F32))
    ga = g * jnp.sum(a8, axis=0, keepdims=True)

    def softmax_b(grp, first_octet):
        wait_kv(k_vm, S_K, grp)
        sb_vm[...] = jnp.zeros((8, SK), F32)

        def body(s, carry):
            for jj in range(4):
                octet_k_then_v(first_octet + s * 4 + jj)
            kh = k_vm[pl.ds(pl.multiple_of((4 * s + grp) * SK, SK), SK), :]
            sb_vm[...] += jax.lax.dot_general(qb_vm[grp * 8 + s].astype(BF16), kh, NT,
                                              preferred_element_type=F32)
            return carry

        jax.lax.fori_loop(0, 8, body, 0)
        sc = sb_vm[...]
        p = jnp.exp(sc - jnp.max(sc, axis=-1, keepdims=True))
        l_vm[grp] = jnp.broadcast_to(jnp.sum(p, axis=-1, keepdims=True), (8, D))
        p_vm[grp] = p.astype(BF16)

    for grp in range(4):
        softmax_b(grp, 48 + 32 * grp)

    omg = 1.0 - g

    def pv_head(grp, s):
        vh = v_vm[ds((4 * s + grp) * SK, SK, SK), :]
        o = jnp.dot(p_vm[grp], vh, preferred_element_type=F32)
        o = o * (omg / l_vm[grp])
        o = jnp.sum(jnp.where(sub == s, o, 0.0), axis=0, keepdims=True)
        o_vm[grp * 8 + s] = jnp.broadcast_to(o, (8, D))

    def pv_group(grp, first_octet):
        wait_kv(v_vm, S_V, grp)

        def body(s, carry):
            for jj in range(4):
                octet_v(first_octet + s * 4 + jj)
            pv_head(grp, s)
            return carry

        jax.lax.fori_loop(0, 8, body, 0)

    def columns(grp):
        base = VPU_GROUPS.index(grp) * 8 * D
        for s in range(8):
            ot_vm[pl.ds(base + s * D, D), :] = jnp.broadcast_to(o_vm[grp * 8 + s][0:1, :], (D, D)).T

    pv_group(0, 48)
    pv_group(1, 80)
    wait_kv(v_vm, S_V, 2)
    v_rest = [functools.partial(octet_v, j) for j in range(112, KV_FULL)]
    v_rest.append(functools.partial(octet_kv_trail, v_hbm, v_vm, S_V))
    for s in range(8):
        for octet in v_rest[2 * s:2 * s + 2]:
            octet()
        pv_head(2, s)
    columns(2)
    for i in range(WO_AHEAD):
        octet_wob(i)
    wait_kv(v_vm, S_V, 3)
    for s in range(8):
        if WO_AHEAD + s < 16:
            octet_wob(WO_AHEAD + s)
        pv_head(3, s)
    columns(3)

    b8 = jnp.zeros((8, M), F32)
    for grp in range(4):
        if grp not in VPU_GROUPS:
            wait_all(wob_vm.at[pl.ds(grp * 8 * D, 8 * D)], S_WOB + grp)
            for slot in range(grp * 8, grp * 8 + 8):
                b8 = b8 + jnp.dot(o_vm[slot].astype(BF16), wob_vm[pl.ds(slot * D, D), :],
                                  preferred_element_type=F32)
    out = ga + b8[0:1, :]
    for grp in VPU_GROUPS:
        for c in range(D // WO_ROWS):
            for s in range(NS):
                wob_copy(grp, s, c).wait()
                w = wob_vm[pl.ds((grp * 8 + s) * D + c * WO_ROWS, WO_ROWS), :].astype(F32)
                r0 = (VPU_GROUPS.index(grp) * 8 + s) * D + c * WO_ROWS
                o_col = jnp.concatenate([ot_vm[pl.ds(r0, WO_ROWS), :]] * (M // D), axis=1)
                out = out + jnp.sum(w * o_col, axis=0, keepdims=True)
    out_ref[...] = out.astype(out_ref.dtype)


def _forward(A_x, A_c_kv, A_w_q, A_w_uk, A_w_uv, A_w_o, B_k_cache, B_v_cache, B_wq, B_wo,
             gate_w, interpret=False):
    hbm = pl.BlockSpec(memory_space=pltpu.HBM)
    out = pl.pallas_call(
        _kernel,
        out_shape=jax.ShapeDtypeStruct((1, M), A_x.dtype),
        in_specs=[hbm] * 11,
        out_specs=pl.BlockSpec(memory_space=pltpu.VMEM),
        scratch_shapes=[
            pltpu.VMEM((1, M), BF16),
            pltpu.VMEM((M,), BF16),
            pltpu.VMEM((1, M), F32),
            pltpu.SMEM((1, M), F32),
            pltpu.VMEM((SK, DC), BF16),
            pltpu.VMEM((M, H, D), BF16),
            pltpu.VMEM((DC, H, D), BF16),
            pltpu.VMEM((DC, H, D), BF16),
            pltpu.VMEM((H * D, M), BF16),
            pltpu.VMEM((H * SK, D), BF16),
            pltpu.VMEM((H * SK, D), BF16),
            pltpu.VMEM((M, H * D), BF16),
            pltpu.VMEM((H * D, M), BF16),
            pltpu.VMEM((H, 8, D), F32),
            pltpu.VMEM((8, SK), F32),
            pltpu.VMEM((H // 8, 8, SK), BF16),
            pltpu.VMEM((H // 8, 8, D), F32),
            pltpu.VMEM((H, 8, D), F32),
            pltpu.VMEM((len(VPU_GROUPS) * 8 * D, D), F32),
            pltpu.VMEM((D, D), F32),
            pltpu.VMEM((SK // KB, H, KB), F32),
            pltpu.VMEM((H // 8, 8, D), F32),
        ],
        compiler_params=pltpu.CompilerParams(vmem_limit_bytes=112 << 20),
        interpret=interpret,
    )(
        A_x.reshape(1, M), gate_w,
        A_c_kv.reshape(SK, DC), A_w_q, A_w_uk, A_w_uv, A_w_o.reshape(H * D, M),
        B_k_cache.reshape(H * SK, D), B_v_cache.reshape(H * SK, D),
        B_wq, B_wo,
    )
    return out.reshape(1, 1, M)


@jax.jit
def pallas_gated_mix__compressed_kv_cla__gqa_block_cached__decode_kernel(
    A_x: jax.Array,
    A_c_kv: jax.Array,
    A_w_q: jax.Array,
    A_w_uk: jax.Array,
    A_w_uv: jax.Array,
    A_w_o: jax.Array,
    B_x: jax.Array,
    B_k_cache: jax.Array,
    B_v_cache: jax.Array,
    B_wq: jax.Array,
    B_wo: jax.Array,
    gate_w: jax.Array,
):
    del B_x
    return _forward(A_x, A_c_kv, A_w_q, A_w_uk, A_w_uv, A_w_o,
                    B_k_cache, B_v_cache, B_wq, B_wo, gate_w)
```

```python
import functools

import jax
import jax.numpy as jnp
from jax.experimental import pallas as pl
from jax.experimental.pallas import tpu as pltpu

H = 32
D = 128
SK = 4096
M = 640
DC = 512
KB = 512
F32 = jnp.float32
BF16 = jnp.bfloat16
NT = (((1,), (1,)), ((), ()))

NS = 8
KV_ROWS = 128
WO_TILES = 16
REGION = 4 * SK
KV_LEAD = 64
KV_FULL = REGION // KV_ROWS - 1

VPU_GROUPS = (2, 3)
WO_AHEAD = 18

NJ = M // D
HEAD_TILES = (D // 8) * NJ
WO_REGION = 4 * HEAD_TILES
WO_LEAD = 8
WO_FULL = WO_REGION // WO_TILES - 1
WO_TAIL0 = 10

S_X, S_GATE, S_XS, S_WQB, S_WQA, S_WUK, S_CKV, S_WUV, S_WOA = range(9)
S_K = 9
S_V = S_K + 4 * NS
S_WOB = S_V + 4 * NS
S_TAIL = S_WOB + 2 * NS
TAIL_PER_REGION = WO_FULL - WO_TAIL0 + 1
N_SEMS = S_TAIL + NS * TAIL_PER_REGION


def _kernel(*refs):
    pl.run_scoped(functools.partial(_body, *refs), pltpu.SemaphoreType.DMA((N_SEMS,)))


def _body(x_hbm, gate_hbm, ckv_hbm, wqa_hbm, wuk_hbm, wuv_hbm, woa_hbm,
          k_hbm, v_hbm, wqb_hbm, wob_hbm,
          out_ref,
          x_vm, gate_vm, xf_vm, x_smem,
          ckv_vm, wqa_vm, wuk_vm, wuv_vm, woa_vm, k_vm, v_vm, wqb_vm, wob_vm,
          qb_vm, sb_vm, p_vm, l_vm, o_vm, ot_vm, y_vm, s_vm, ctx_vm, sems):
    scale = D ** -0.5

    def start(src, dst, sem, thread):
        pltpu.make_async_copy(src, dst, sems.at[sem]).start(thread)

    def wait_all(buf, sem):
        pltpu.make_async_copy(buf, buf, sems.at[sem]).wait()

    def ds(start_, size, align):
        return pl.ds(start_ if isinstance(start_, int) else pl.multiple_of(start_, align), size)

    def wqb_piece(q, strip, col0, cols):
        idx = (ds(q * 160 + strip * 8, 8, 8), pl.ds(col0, cols))
        start(wqb_hbm.at[idx], wqb_vm.at[idx], S_WQB, 0)

    def wqa_piece(q, i):
        idx = ds(q * 160 + i * 4, 4, 4)
        start(wqa_hbm.at[idx], wqa_vm.at[idx], S_WQA, 1)

    def w1_lead():
        for q in range(4):
            wqb_piece(q, 0, 0, 1024)

    def w1_strip(r):
        for q in range(4):
            wqb_piece(q, r, 1024, 2048)
            wqa_piece(q, 2 * r)
        for q in range(4):
            wqb_piece(q, r, 3072, 1024)
            wqa_piece(q, 2 * r + 1)

        @pl.when(r + 1 < 20)
        def _():
            for q in range(4):
                wqb_piece(q, r + 1, 0, 1024)

    def octet_w2(i):
        for q in range(4):
            idx = ds(q * 128 + i * 4, 4, 4)
            start(wuk_hbm.at[idx], wuk_vm.at[idx], S_WUK, 0)
            idx = ds(q * 1024 + i * 32, 32, 32)
            start(ckv_hbm.at[idx], ckv_vm.at[idx], S_CKV, 1)

    def octet_w3(i):
        for q in range(4):
            idx = ds(q * 128 + i * 4, 4, 4)
            start(wuv_hbm.at[idx], wuv_vm.at[idx], S_WUV, 0)
            idx = ds(q * 640 + i * WO_TILES, WO_TILES, WO_TILES)
            start(woa_hbm.at[idx], woa_vm.at[idx], S_WOA, 1)

    def woa_rest():
        for i in range(32, 40):
            for q in range(4):
                idx = pl.ds(q * 640 + i * WO_TILES, WO_TILES)
                start(woa_hbm.at[idx], woa_vm.at[idx], S_WOA, q % 2)

    def octet_kv(hbm, vm, sem0, j):
        for s in range(NS):
            idx = ds(s * REGION + KV_LEAD + j * KV_ROWS, KV_ROWS, 8)
            start(hbm.at[idx], vm.at[idx], sem0 + 4 * s + j // (SK // KV_ROWS), s % 2)

    def octet_kv_lead(hbm, vm, sem0):
        for s in range(NS):
            idx = pl.ds(s * REGION, KV_LEAD)
            start(hbm.at[idx], vm.at[idx], sem0 + 4 * s, s % 2)

    def octet_kv_trail(hbm, vm, sem0):
        for s in range(NS):
            idx = pl.ds(s * REGION + KV_LEAD + KV_FULL * KV_ROWS, KV_ROWS - KV_LEAD)
            start(hbm.at[idx], vm.at[idx], sem0 + 4 * s + 3, s % 2)

    def wait_kv(vm, sem0, grp):
        r0 = 0 if grp == 0 else grp * SK + KV_LEAD
        r1 = REGION if grp == 3 else (grp + 1) * SK + KV_LEAD
        for s in range(NS):
            wait_all(vm.at[pl.ds(s * REGION + r0, r1 - r0)], sem0 + 4 * s + grp)

    octet_k = functools.partial(octet_kv, k_hbm, k_vm, S_K)
    octet_v = functools.partial(octet_kv, v_hbm, v_vm, S_V)

    def octet_k_then_v(u):
        @pl.when(u < KV_FULL)
        def _():
            octet_k(u)

        @pl.when(u == KV_FULL)
        def _():
            octet_kv_trail(k_hbm, k_vm, S_K)
            octet_kv_lead(v_hbm, v_vm, S_V)

        @pl.when(u > KV_FULL)
        def _():
            octet_v(u - KV_FULL - 1)

    def wob_copy(s, k):
        if k < 0:
            t0, n = 0, WO_LEAD
        elif k < WO_FULL:
            t0, n = WO_LEAD + k * WO_TILES, WO_TILES
        else:
            t0, n = WO_LEAD + WO_FULL * WO_TILES, WO_TILES - WO_LEAD
        idx = pl.ds(s * WO_REGION + t0, n)
        if k >= WO_TAIL0:
            sem = S_TAIL + s * TAIL_PER_REGION + (k - WO_TAIL0)
        else:
            sem = S_WOB + 2 * s + t0 // HEAD_TILES
        return pltpu.make_async_copy(wob_hbm.at[idx], wob_vm.at[idx], sems.at[sem]), t0, n

    def octet_wob(i):
        for s in range(NS):
            wob_copy(s, i - 1)[0].start(s % 2)

    def wait_wob(grp):
        t0 = 0 if grp == 0 else grp * HEAD_TILES + WO_LEAD
        t1 = (grp + 1) * HEAD_TILES + WO_LEAD
        for s in range(NS):
            wait_all(wob_vm.at[pl.ds(s * WO_REGION + t0, t1 - t0)], S_WOB + 2 * s + grp)

    def wo_tile(vm, head, j):
        return jnp.concatenate([vm[head * HEAD_TILES + u * NJ + j] for u in range(D // 8)], axis=0)

    def pump(octet, first, count):
        def body(i, carry):
            octet(first + 2 * i)
            octet(first + 2 * i + 1)
            return carry
        jax.lax.fori_loop(0, count // 2, body, 0)

    sub = jax.lax.broadcasted_iota(jnp.int32, (8, D), 0)
    row = jax.lax.broadcasted_iota(jnp.int32, (H, D), 0)
    lane = jax.lax.broadcasted_iota(jnp.int32, (H, D), 1)
    diag = row == lane % H

    start(x_hbm, x_vm, S_X, 0)
    start(gate_hbm, gate_vm, S_GATE, 0)
    w1_lead()
    jax.lax.fori_loop(0, 20, lambda r, carry: (w1_strip(r), carry)[1], 0)
    pump(octet_w2, 0, 14)

    pltpu.make_async_copy(x_hbm, x_vm, sems.at[S_X]).wait()
    pltpu.make_async_copy(gate_hbm, gate_vm, sems.at[S_GATE]).wait()
    xf = x_vm[...].astype(F32)
    xf_vm[...] = xf
    x_to_smem = pltpu.make_async_copy(xf_vm, x_smem, sems.at[S_XS])
    x_to_smem.start()
    gw = gate_vm[...].astype(F32).reshape(1, M)
    z = jnp.sum(xf * gw, axis=-1, keepdims=True)
    g = 1.0 / (1.0 + jnp.exp(-z))

    wait_all(wqb_vm, S_WQB)
    x8 = jnp.broadcast_to(x_vm[...], (8, M))
    qb = jnp.dot(x8, wqb_vm[...], preferred_element_type=F32) * scale
    for slot in range(H):
        h = 4 * (slot % 8) + slot // 8
        qb_vm[slot] = jnp.where(sub == slot % 8, qb[:, h * D:(h + 1) * D], 0.0)

    x_to_smem.wait()
    wait_all(wqa_vm, S_WQA)

    def qa_outer(i, acc):
        octet_w2(14 + i)

        def qa_inner(j, acc):
            for jj in range(8):
                m = i * 64 + j * 8 + jj
                acc = acc + wqa_vm[m].astype(F32) * x_smem[0, m]
            return acc

        return jax.lax.fori_loop(0, 8, qa_inner, acc)

    qa = jax.lax.fori_loop(0, M // 64, qa_outer, jnp.zeros((H, D), F32)).astype(BF16)
    pump(octet_w2, 24, 8)
    pump(octet_w3, 0, 14)

    wait_all(wuk_vm, S_WUK)

    def qlat_body(i, carry):
        octet_w3(14 + i)
        rows8 = jnp.zeros((8, D), F32)
        for j in range(8):
            t = i * 8 + j
            w = jnp.concatenate([wuk_vm[cc * D + t] for cc in range(DC // D)], axis=0)
            prod = jax.lax.dot_general(qa, w, NT, preferred_element_type=F32)
            picked = jnp.sum(jnp.where(diag, prod, 0.0), axis=0, keepdims=True)
            rows8 = jnp.where(sub == j, picked, rows8)
        y_vm[pl.ds(pl.multiple_of(i * 8, 8), 8), :] = rows8
        return carry

    jax.lax.fori_loop(0, D // 8, qlat_body, 0)
    octet_w3(30)
    octet_w3(31)
    woa_rest()
    yt = y_vm[...].T
    qlat = jnp.concatenate([yt[cc * H:(cc + 1) * H, :] for cc in range(DC // D)], axis=1)
    qlat = (qlat * scale).astype(BF16)

    wait_all(ckv_vm, S_CKV)
    octet_kv_lead(k_hbm, k_vm, S_K)

    def score_body(i, mx):
        octet_k(i)
        c = ckv_vm[pl.ds(pl.multiple_of(i * KB, KB), KB), :]
        s = jax.lax.dot_general(qlat, c, NT, preferred_element_type=F32)
        s_vm[i] = s
        return jnp.maximum(mx, s)

    mx = jax.lax.fori_loop(0, SK // KB, score_body, jnp.full((H, KB), -jnp.inf, F32))
    ma = jnp.max(mx, axis=-1, keepdims=True)

    def ctx_lat_body(i, carry):
        octet_k(8 + i)
        acc, lsum = carry
        p = jnp.exp(s_vm[i] - ma)
        c = ckv_vm[pl.ds(pl.multiple_of(i * KB, KB), KB), :]
        return acc + jnp.dot(p.astype(BF16), c, preferred_element_type=F32), lsum + p

    clat, lsum = jax.lax.fori_loop(
        0, SK // KB, ctx_lat_body, (jnp.zeros((H, DC), F32), jnp.zeros((H, KB), F32)))
    clat = clat / jnp.sum(lsum, axis=-1, keepdims=True)

    wait_all(wuv_vm, S_WUV)
    u = jnp.concatenate([clat[:, cc * D:(cc + 1) * D] for cc in range(DC // D)], axis=0)
    y_vm[...] = u.T

    def ctx_body(i, acc):
        octet_k(16 + i)
        rows8 = y_vm[pl.ds(pl.multiple_of(i * 8, 8), 8), :]
        for j in range(8):
            t = i * 8 + j
            w = jnp.concatenate([wuv_vm[cc * D + t] for cc in range(DC // D)], axis=0)
            lhs = jnp.where(diag, jnp.broadcast_to(rows8[j:j + 1, :], (H, D)), 0.0)
            acc = acc + jnp.dot(lhs.astype(BF16), w, preferred_element_type=F32)
        return acc

    ctx = jax.lax.fori_loop(0, D // 8, ctx_body, jnp.zeros((H, D), F32))
    for i in range(H // 8):
        ctx_vm[i] = ctx[i * 8:(i + 1) * 8, :]

    wait_all(woa_vm, S_WOA)

    def proj_a_body(i, acc):
        octet_k(32 + i)
        for jj in range(2):
            h = 2 * i + jj
            lhs = jnp.where(sub == h % 8, ctx_vm[h // 8], 0.0).astype(BF16)
            acc = tuple(acc[j] + jnp.dot(lhs, wo_tile(woa_vm, h, j), preferred_element_type=F32)
                        for j in range(NJ))
        return acc

    a8 = jax.lax.fori_loop(0, H // 2, proj_a_body, (jnp.zeros((8, D), F32),) * NJ)
    ga = g * jnp.sum(jnp.concatenate(a8, axis=1), axis=0, keepdims=True)

    def softmax_b(grp, first_octet):
        wait_kv(k_vm, S_K, grp)
        sb_vm[...] = jnp.zeros((8, SK), F32)

        def body(s, carry):
            for jj in range(4):
                octet_k_then_v(first_octet + s * 4 + jj)
            kh = k_vm[pl.ds(pl.multiple_of((4 * s + grp) * SK, SK), SK), :]
            sb_vm[...] += jax.lax.dot_general(qb_vm[grp * 8 + s].astype(BF16), kh, NT,
                                              preferred_element_type=F32)
            return carry

        jax.lax.fori_loop(0, 8, body, 0)
        sc = sb_vm[...]
        p = jnp.exp(sc - jnp.max(sc, axis=-1, keepdims=True))
        l_vm[grp] = jnp.broadcast_to(jnp.sum(p, axis=-1, keepdims=True), (8, D))
        p_vm[grp] = p.astype(BF16)

    for grp in range(4):
        softmax_b(grp, 48 + 32 * grp)

    omg = 1.0 - g

    def pv_head(grp, s):
        vh = v_vm[ds((4 * s + grp) * SK, SK, SK), :]
        o = jnp.dot(p_vm[grp], vh, preferred_element_type=F32)
        o = o * (omg / l_vm[grp])
        o = jnp.sum(jnp.where(sub == s, o, 0.0), axis=0, keepdims=True)
        o_vm[grp * 8 + s] = jnp.broadcast_to(o, (8, D))

    def pv_group(grp, first_octet):
        wait_kv(v_vm, S_V, grp)

        def body(s, carry):
            for jj in range(4):
                octet_v(first_octet + s * 4 + jj)
            pv_head(grp, s)
            return carry

        jax.lax.fori_loop(0, 8, body, 0)

    def columns(grp):
        base = VPU_GROUPS.index(grp) * 8 * D
        for s in range(8):
            ot_vm[pl.ds(base + s * D, D), :] = jnp.broadcast_to(o_vm[grp * 8 + s][0:1, :], (D, D)).T

    pv_group(0, 48)
    pv_group(1, 80)
    wait_kv(v_vm, S_V, 2)
    v_rest = [functools.partial(octet_v, j) for j in range(112, KV_FULL)]
    v_rest.append(functools.partial(octet_kv_trail, v_hbm, v_vm, S_V))
    for s in range(8):
        for octet in v_rest[2 * s:2 * s + 2]:
            octet()
        pv_head(2, s)
    columns(2)
    for i in range(WO_AHEAD):
        octet_wob(i)
    wait_kv(v_vm, S_V, 3)
    for s in range(8):
        if WO_AHEAD + s < WO_FULL + 2:
            octet_wob(WO_AHEAD + s)
        pv_head(3, s)
    columns(3)

    b8 = [jnp.zeros((8, D), F32)] * NJ
    for grp in (0, 1):
        wait_wob(grp)
        for s in range(NS):
            lhs = o_vm[grp * 8 + s].astype(BF16)
            b8 = [b8[j] + jnp.dot(lhs, wo_tile(wob_vm, 4 * s + grp, j), preferred_element_type=F32)
                  for j in range(NJ)]
    base = ga + jnp.concatenate([b[0:1, :] for b in b8], axis=1)

    acc = [jnp.zeros((8, D), F32)] * NJ

    def fold(acc, s, t0, n):
        acc = list(acc)
        for t in range(t0, t0 + n):
            grp, u, j = t // HEAD_TILES, (t % HEAD_TILES) // NJ, t % NJ
            r0 = (VPU_GROUPS.index(grp) * 8 + s) * D + u * 8
            acc[j] = acc[j] + wob_vm[s * WO_REGION + t].astype(F32) * ot_vm[pl.ds(r0, 8), :]
        return acc

    for s in range(NS):
        acc = fold(acc, s, 2 * HEAD_TILES, WO_LEAD + WO_TAIL0 * WO_TILES - 2 * HEAD_TILES)
    for k in range(WO_TAIL0, WO_FULL + 1):
        for s in range(NS):
            copy, t0, n = wob_copy(s, k)
            copy.wait()
            acc = fold(acc, s, t0, n)
    out = base + jnp.concatenate([jnp.sum(a, axis=0, keepdims=True) for a in acc], axis=1)
    out_ref[...] = out.astype(out_ref.dtype)


def _tiles(w):
    return w.reshape(H * D // 8, 8, NJ, D).transpose(0, 2, 1, 3).reshape(H * HEAD_TILES, 8, D)


def _forward(A_x, A_c_kv, A_w_q, A_w_uk, A_w_uv, A_w_o, B_k_cache, B_v_cache, B_wq, B_wo,
             gate_w, interpret=False):
    hbm = pl.BlockSpec(memory_space=pltpu.HBM)
    out = pl.pallas_call(
        _kernel,
        out_shape=jax.ShapeDtypeStruct((1, M), A_x.dtype),
        in_specs=[hbm] * 11,
        out_specs=pl.BlockSpec(memory_space=pltpu.VMEM),
        scratch_shapes=[
            pltpu.VMEM((1, M), BF16),
            pltpu.VMEM((M,), BF16),
            pltpu.VMEM((1, M), F32),
            pltpu.SMEM((1, M), F32),
            pltpu.VMEM((SK, DC), BF16),
            pltpu.VMEM((M, H, D), BF16),
            pltpu.VMEM((DC, H, D), BF16),
            pltpu.VMEM((DC, H, D), BF16),
            pltpu.VMEM((H * HEAD_TILES, 8, D), BF16),
            pltpu.VMEM((H * SK, D), BF16),
            pltpu.VMEM((H * SK, D), BF16),
            pltpu.VMEM((M, H * D), BF16),
            pltpu.VMEM((H * HEAD_TILES, 8, D), BF16),
            pltpu.VMEM((H, 8, D), F32),
            pltpu.VMEM((8, SK), F32),
            pltpu.VMEM((H // 8, 8, SK), BF16),
            pltpu.VMEM((H // 8, 8, D), F32),
            pltpu.VMEM((H, 8, D), F32),
            pltpu.VMEM((len(VPU_GROUPS) * 8 * D, D), F32),
            pltpu.VMEM((D, D), F32),
            pltpu.VMEM((SK // KB, H, KB), F32),
            pltpu.VMEM((H // 8, 8, D), F32),
        ],
        compiler_params=pltpu.CompilerParams(vmem_limit_bytes=112 << 20),
        interpret=interpret,
    )(
        A_x.reshape(1, M), gate_w,
        A_c_kv.reshape(SK, DC), A_w_q, A_w_uk, A_w_uv, _tiles(A_w_o.reshape(H * D, M)),
        B_k_cache.reshape(H * SK, D), B_v_cache.reshape(H * SK, D),
        B_wq, _tiles(B_wo),
    )
    return out.reshape(1, 1, M)


@jax.jit
def pallas_gated_mix__compressed_kv_cla__gqa_block_cached__decode_kernel(
    A_x: jax.Array,
    A_c_kv: jax.Array,
    A_w_q: jax.Array,
    A_w_uk: jax.Array,
    A_w_uv: jax.Array,
    A_w_o: jax.Array,
    B_x: jax.Array,
    B_k_cache: jax.Array,
    B_v_cache: jax.Array,
    B_wq: jax.Array,
    B_wo: jax.Array,
    gate_w: jax.Array,
):
    del B_x
    return _forward(A_x, A_c_kv, A_w_q, A_w_uk, A_w_uv, A_w_o,
                    B_k_cache, B_v_cache, B_wq, B_wo, gate_w)
```
